```python
import jax
import jax.numpy as jnp

def _softmax(x, axis=-1):
    return jax.nn.softmax(x, axis=axis)

def _gelu(x):
    return jax.nn.gelu(x, approximate=True)

def _silu(x):
    return jax.nn.silu(x)

def _sigmoid(x):
    return jax.nn.sigmoid(x)

def _layernorm(x, axis=-1, eps=1e-05):
    m = jnp.mean(x, axis=axis, keepdims=True)
    v = jnp.var(x, axis=axis, keepdims=True)
    return (x - m) / jnp.sqrt(v + eps)

def _scatter_add(tgt, idx, src, axis=0):
    return tgt.at[idx].add(src)

def _segment_sum(src, seg, n):
    return jax.ops.segment_sum(src, seg, n)

class _Rng:

    def __init__(self, key):
        self._k = key

    def _next(self):
        self._k, sub = jax.random.split(self._k)
        return sub

    def normal(self, shape):
        return jax.random.normal(self._next(), shape, dtype=jnp.bfloat16)

    def randint(self, lo, hi, shape):
        return jax.random.randint(self._next(), shape, lo, hi, dtype=jnp.int32)

    def uniform(self, shape, lo=0.0, hi=1.0):
        return jax.random.uniform(self._next(), shape, jnp.bfloat16, lo, hi)

    def permutation(self, n):
        return jax.random.permutation(self._next(), n)
kernel_name = 'concat_heads__sliding_local_dilated__memory_aug_recurrent_mem_tr__prompt'

def setup_inputs():
    _rng = _Rng(jax.random.key(int.from_bytes(__import__("os").urandom(4), "little")))
    _w = lambda a: (lambda t: t.astype(jnp.bfloat16) if jnp.issubdtype(t.dtype, jnp.floating) else t)(jnp.asarray(a))

    def _A_setup():
        B, S, D = (1, 2048, 640)
        return {'x': _w((lambda *s: _rng.normal(s) * 0.05)(B, S, D)), 'wqkv': _w((lambda *s: _rng.normal(s) * 0.05)(D, 3 * D)), 'wo': _w((lambda *s: _rng.normal(s) * 0.05)(D, D))}
    _A_in = _A_setup()

    def _B_setup():
        B, S, Dm = (1, 2048, 640)
        H, Dh = (32, 192)
        M, seg = (8, 32)
        seg = min(seg, S)
        S = S // seg * seg
        return {'x': _w((lambda *s: _rng.normal(s) * 0.05)(B, S, Dm)), 'mem0': _w((lambda *s: _rng.normal(s) * 0.05)(B, M, Dm)), 'Wq': _w((lambda *s: _rng.normal(s) * 0.05)(Dm, H, Dh) * Dm ** (-0.5)), 'Wk': _w((lambda *s: _rng.normal(s) * 0.05)(Dm, H, Dh) * Dm ** (-0.5)), 'Wv': _w((lambda *s: _rng.normal(s) * 0.05)(Dm, H, Dh) * Dm ** (-0.5)), 'Wo': _w((lambda *s: _rng.normal(s) * 0.05)(H, Dh, Dm) * (H * Dh) ** (-0.5)), 'seg_len': seg}
    _B_in = _B_setup()
    return {'A_x': _A_in['x'], 'A_wqkv': _A_in['wqkv'], 'A_wo': _A_in['wo'], 'B_x': _B_in['x'], 'B_mem0': _B_in['mem0'], 'B_Wq': _B_in['Wq'], 'B_Wk': _B_in['Wk'], 'B_Wv': _B_in['Wv'], 'B_Wo': _B_in['Wo'], 'B_seg_len': _B_in['seg_len']}

def reference(A_x, A_wqkv, A_wo, B_x, B_mem0, B_Wq, B_Wk, B_Wv, B_Wo, B_seg_len):

    def _A_ref(x, wqkv, wo):
        B, S, D = x.shape
        H = 32
        Dh = D // H
        W, dil = (8, 2)
        qkv = (lambda x, *d: x.transpose(*d))((x @ wqkv).reshape(B, S, 3, H, Dh), 2, 0, 3, 1, 4)
        q, k, v = (qkv[0], qkv[1], qkv[2])
        scale = Dh ** (-0.5)
        pos = jnp.arange(S)
        off = jnp.arange(W) * dil
        idx = pos[:, None] - off[None, :]
        mask = idx >= 0
        idx_c = jnp.where(mask, idx, 0).reshape(-1)
        kg = k[:, :, idx_c, :].reshape(B, H, S, W, Dh)
        vg = v[:, :, idx_c, :].reshape(B, H, S, W, Dh)
        logits = jnp.einsum('bhsd,bhswd->bhsw', q, kg) * scale
        logits = jnp.where(mask[None, None, :, :], logits, -1000000000.0)
        attn = _softmax(logits, axis=-1)
        o = jnp.einsum('bhsw,bhswd->bhsd', attn, vg)
        return (lambda x, *d: x.transpose(*d))(o, 0, 2, 1, 3).reshape(B, S, D) @ wo

    def _B_ref(x, mem0, Wq, Wk, Wv, Wo, seg_len):
        B, S, Dm = x.shape
        H, Dh = (Wq.shape[1], Wq.shape[2])
        M = mem0.shape[1]
        scale = Dh ** (-0.5)
        n_seg = S // seg_len
        L = M + seg_len
        idx = jnp.arange(L)
        mask = (idx[:, None] < M) | (idx[:, None] >= idx[None, :])
        mem = mem0
        outs = []
        for s in range(n_seg):
            xs = x[:, s * seg_len:(s + 1) * seg_len, :].copy()
            h = jnp.concatenate([mem, xs], axis=1)
            q = jnp.einsum('btd,dhe->bhte', h, Wq)
            k = jnp.einsum('btd,dhe->bhte', h, Wk)
            v = jnp.einsum('btd,dhe->bhte', h, Wv)
            scores = jnp.einsum('bhqe,bhke->bhqk', q, k) * scale
            scores = jnp.where(mask[None, None], scores, -1000000000.0)
            p = _softmax(scores, axis=-1)
            o = jnp.einsum('bhqk,bhke->bhqe', p, v)
            o = jnp.einsum('bhte,hed->btd', o, Wo)
            mem = o[:, :M, :].copy()
            outs.append(o[:, M:, :])
        return jnp.concatenate(outs, axis=1)
    a = _A_ref(A_x, A_wqkv, A_wo)
    b = _B_ref(B_x, B_mem0, B_Wq, B_Wk, B_Wv, B_Wo, B_seg_len)
    return jnp.concatenate([a, b], axis=-1)
```

```python
import functools

import jax
import jax.numpy as jnp
from jax import lax
import jax.experimental.pallas as pl
import jax.experimental.pallas.tpu as pltpu

BF16 = jnp.bfloat16
F32 = jnp.float32
U32 = jnp.uint32

_NN = (((1,), (0,)), ((), ()))
_NT = (((1,), (1,)), ((), ()))

LANES = 128
NEG = -1000000000.0

A_HEADS = 32
A_WIN = 8
A_DIL = 2
A_HALO = 16
A_ROWS = 128


def _dot(a, b, dn=_NN):
    return lax.dot_general(a, b, dn, preferred_element_type=F32)


def _pack(x):
    return pltpu.bitcast(x, U32)


def _unpack(x):
    return pltpu.bitcast(x, BF16)


def _kernel(
    xa_hbm, wqkv_hbm, woa_hbm, xb_hbm, mem_hbm, wq_hbm, wk_hbm, wv_hbm, wo_hbm,
    out_hbm,
    xa_v, wqkv_raw, woa_raw, wqkv_p, woa_p, set_e, set_o, outa_v,
    xb_v, mem_v, w_raw, wo_raw, wt, wo_p, outb_v,
    sem_a, sem_w, sem_o,
    *, seg, head_dim,
):
    S, D = xa_v.shape
    M = mem_v.shape[0]
    L = M + seg
    PW = 2 * head_dim
    NP = wt.shape[1]
    NT = D // LANES
    R = A_ROWS
    n_it = S // (2 * R)
    ppi = NP // n_it

    a_copies = [
        pltpu.make_async_copy(
            wqkv_hbm.at[:, pl.ds(i * D, D)], wqkv_raw.at[i], sem_a.at[i])
        for i in range(3)
    ] + [
        pltpu.make_async_copy(xa_hbm, xa_v, sem_a.at[3]),
        pltpu.make_async_copy(woa_hbm, woa_raw, sem_a.at[4]),
        pltpu.make_async_copy(mem_hbm, mem_v, sem_a.at[5]),
        pltpu.make_async_copy(xb_hbm, xb_v, sem_a.at[6]),
    ]

    def w_copies(g):
        rows = pl.ds(g * ppi * PW, ppi * PW)
        return [
            pltpu.make_async_copy(wq_hbm.at[rows], w_raw.at[0, rows], sem_w.at[4 * g]),
            pltpu.make_async_copy(wk_hbm.at[rows], w_raw.at[1, rows], sem_w.at[4 * g + 1]),
            pltpu.make_async_copy(wv_hbm.at[rows], w_raw.at[2, rows], sem_w.at[4 * g + 2]),
            pltpu.make_async_copy(wo_hbm.at[rows], wo_raw.at[rows], sem_w.at[4 * g + 3]),
        ]

    for c in a_copies[:5]:
        c.start()
    for g in range(n_it):
        for c in w_copies(g):
            c.start()
    for c in a_copies[5:]:
        c.start()

    def wait_group(g):
        for c in w_copies(g):
            c.wait()

    def relayout_group(g):
        for jj in range(ppi):
            j = g * ppi + jj
            rows = pl.ds(pl.multiple_of(j * PW, PW), PW)
            for m in range(3):
                wt[m, j] = _pack(w_raw[m, rows, :].T)
            wo_p[j] = _pack(wo_raw[rows, :])

    dh = D // A_HEADS
    r_i = lax.broadcasted_iota(jnp.int32, (D, D), 0)
    c_i = lax.broadcasted_iota(jnp.int32, (D, D), 1)
    perm = jnp.where(r_i == (c_i % A_HEADS) * dh + c_i // A_HEADS, 1.0, 0.0).astype(BF16)
    for i in range(3):
        a_copies[i].wait()
        wqkv_p[:, i * D:(i + 1) * D] = _pack(_dot(wqkv_raw[i], perm).astype(BF16))
    perm_t = jnp.where(c_i == (r_i % A_HEADS) * dh + r_i // A_HEADS, 1.0, 0.0).astype(BF16)
    a_copies[3].wait()
    a_copies[4].wait()
    woa_p[...] = _pack(_dot(perm_t, woa_raw[...]).astype(BF16))

    a_scale = dh ** -0.5

    def a_proj(c, dst):
        x = xa_v[pl.ds(pl.multiple_of(c * R, R), R), :]
        qkv = _dot(x, _unpack(wqkv_p[...]))
        for t in range(3 * NT):
            dst[t, A_HALO:, :] = qkv[:, t * LANES:(t + 1) * LANES]

    def a_halo(src, dst):
        for t in range(NT, 3 * NT):
            dst[t, :A_HALO, :] = src[t, R:, :]

    def a_attn(c, src, first):
        q = [src[t, A_HALO:, :] for t in range(NT)]
        logits = []
        for w in range(A_WIN):
            lo = A_HALO - A_DIL * w
            s = q[0] * src[NT, lo:lo + R, :]
            for t in range(1, NT):
                s = s + q[t] * src[NT + t, lo:lo + R, :]
            s = s + pltpu.roll(s, 2 * A_HEADS, 1)
            s = s + pltpu.roll(s, A_HEADS, 1)
            s = s * a_scale
            if first and w > 0:
                row = lax.broadcasted_iota(jnp.int32, (R, LANES), 0)
                s = jnp.where(row >= A_DIL * w, s, NEG)
            logits.append(s)
        mx = functools.reduce(jnp.maximum, logits)
        e = [jnp.exp(s - mx) for s in logits]
        inv = 1.0 / functools.reduce(jnp.add, e)
        p = [x * inv for x in e]
        o = []
        for t in range(NT):
            acc = p[0] * src[2 * NT + t, A_HALO:, :]
            for w in range(1, A_WIN):
                lo = A_HALO - A_DIL * w
                acc = acc + p[w] * src[2 * NT + t, lo:lo + R, :]
            o.append(acc)
        return jnp.concatenate(o, axis=1).astype(BF16)

    def a_out(c, o):
        outa_v[pl.ds(pl.multiple_of(c * R, R), R), :] = _dot(
            o, _unpack(woa_p[...])).astype(BF16)

    a_proj(0, set_e)
    for t in range(NT, 3 * NT):
        set_e[t, :A_HALO, :] = jnp.broadcast_to(
            set_e[t, A_HALO:A_HALO + 1, :], (A_HALO, LANES))
    a_halo(set_e, set_o)
    o = a_attn(0, set_e, True)
    a_proj(1, set_o)
    a_out(0, o)

    def a_body(i, relayout):
        if relayout:
            wait_group(i - 2)
        a_halo(set_o, set_e)
        o = a_attn(2 * i - 1, set_o, False)
        a_proj(2 * i, set_e)
        a_out(2 * i - 1, o)
        a_halo(set_e, set_o)
        o = a_attn(2 * i, set_e, False)
        a_proj(2 * i + 1, set_o)
        a_out(2 * i, o)
        if relayout:
            relayout_group(i - 2)

    a_body(1, False)

    def a_loop(i, carry):
        a_body(i, True)
        return carry

    lax.fori_loop(2, n_it, a_loop, 0)
    a_out(2 * n_it - 1, a_attn(2 * n_it - 1, set_o, False))

    def tail_loop(g, carry):
        wait_group(g)
        relayout_group(g)
        return carry

    lax.fori_loop(n_it - 2, n_it, tail_loop, 0)
    a_copies[5].wait()
    a_copies[6].wait()

    outa_copy = pltpu.make_async_copy(outa_v, out_hbm.at[:, pl.ds(0, D)], sem_o.at[0])
    outa_copy.start()

    b_scale = head_dim ** -0.5

    order = []
    for t in range(NP):
        order.append(("q", t))
        order.append(("k", t))
        order.append(("v", t))
        if t >= 1:
            order.append(("pv", t - 1))
        order.append(("s", t))
        if t >= 5:
            order.append(("o", t - 5))
    order += [("o", NP - 5), ("o", NP - 4), ("o", NP - 3), ("pv", NP - 1),
              ("o", NP - 2), ("o", NP - 1)]

    def b_step(s, mem):
        r0 = pl.multiple_of(s * seg, seg)
        h = jnp.concatenate([mem, xb_v[pl.ds(r0, seg), :].astype(F32)], axis=0)
        lane = lax.broadcasted_iota(jnp.int32, (L, LANES), 1)
        row = lax.broadcasted_iota(jnp.int32, (L, LANES), 0)
        is_a = lane < L
        is_b = (lane >= L) & (lane < 2 * L)
        visible = (row < M) | (row >= jnp.where(is_a, lane, lane - L))
        feat_a = lax.broadcasted_iota(jnp.int32, (L, PW), 1) < head_dim

        def block_diag(t):
            return jnp.concatenate(
                [jnp.where(feat_a, t, 0.0), jnp.where(feat_a, 0.0, t),
                 jnp.zeros((LANES - 2 * L, PW), F32)], axis=0).astype(BF16)

        q, k, v, p, o = {}, {}, {}, {}, {}
        acc = None
        for op, j in order:
            if op == "q":
                q[j] = _dot(h, _unpack(wt[0, j]))
            elif op == "k":
                k[j] = _dot(h, _unpack(wt[1, j]))
            elif op == "v":
                v[j] = _dot(h, _unpack(wt[2, j]))
            elif op == "s":
                sc = _dot(q[j], block_diag(k[j]), _NT) * b_scale
                sc = jnp.where(visible, sc, NEG)
                m_a = jnp.max(jnp.where(is_a, sc, -jnp.inf), axis=1, keepdims=True)
                m_b = jnp.max(jnp.where(is_b, sc, -jnp.inf), axis=1, keepdims=True)
                e = jnp.exp(sc - jnp.where(is_a, m_a, m_b))
                e_a = jnp.where(is_a, e, 0.0)
                e_b = jnp.where(is_b, e, 0.0)
                l_a = jnp.sum(e_a, axis=1, keepdims=True)
                l_b = jnp.sum(e_b, axis=1, keepdims=True)
                p[j] = (e_a + e_b) / jnp.where(is_a, l_a, l_b)
            elif op == "pv":
                o[j] = _dot(p[j], block_diag(v[j]))
            else:
                d = _dot(o[j], _unpack(wo_p[j]))
                acc = d if acc is None else acc + d
        outb_v[pl.ds(r0, seg), :] = acc[M:].astype(BF16)
        return acc[:M]

    n_seg = S // seg
    n_out = sem_o.shape[0] - 1
    spo = n_seg // n_out

    def outb_copy(i):
        rows = pl.ds(pl.multiple_of(i * spo * seg, spo * seg), spo * seg)
        return pltpu.make_async_copy(
            outb_v.at[rows], out_hbm.at[rows, pl.ds(D, D)], sem_o.at[i + 1])

    def b_outer(i, mem):
        mem = lax.fori_loop(i * spo, (i + 1) * spo, b_step, mem)
        outb_copy(i).start()
        return mem

    lax.fori_loop(0, n_out, b_outer, mem_v[...].astype(F32))

    outa_copy.wait()
    for i in range(n_out):
        outb_copy(i).wait()


@functools.partial(jax.jit, static_argnames=("B_seg_len",))
def pallas_concat_heads__sliding_local_dilated__memory_aug_recurrent_mem_tr__prompt_kernel(
    A_x: jax.Array,
    A_wqkv: jax.Array,
    A_wo: jax.Array,
    B_x: jax.Array,
    B_mem0: jax.Array,
    B_Wq: jax.Array,
    B_Wk: jax.Array,
    B_Wv: jax.Array,
    B_Wo: jax.Array,
    B_seg_len: int,
):
    _, S, D = A_x.shape
    _, H, Dh = B_Wq.shape
    M = B_mem0.shape[1]
    HD = H * Dh
    NP = H // 2
    PW = 2 * Dh
    n_groups = S // (2 * A_ROWS)
    n_out = 8

    def heads_major(w):
        return w.transpose(1, 2, 0).reshape(HD, D)

    qkv_set = pltpu.VMEM((3 * D // LANES, A_HALO + A_ROWS, LANES), F32)
    out = pl.pallas_call(
        functools.partial(_kernel, seg=B_seg_len, head_dim=Dh),
        out_shape=jax.ShapeDtypeStruct((S, 2 * D), BF16),
        in_specs=[pl.BlockSpec(memory_space=pltpu.HBM)] * 9,
        out_specs=pl.BlockSpec(memory_space=pltpu.HBM),
        scratch_shapes=[
            pltpu.VMEM((S, D), BF16),
            pltpu.VMEM((3, D, D), BF16),
            pltpu.VMEM((D, D), BF16),
            pltpu.VMEM((D // 2, 3 * D), U32),
            pltpu.VMEM((D // 2, D), U32),
            qkv_set,
            qkv_set,
            pltpu.VMEM((S, D), BF16),
            pltpu.VMEM((S, D), BF16),
            pltpu.VMEM((M, D), BF16),
            pltpu.VMEM((3, HD, D), BF16),
            pltpu.VMEM((HD, D), BF16),
            pltpu.VMEM((3, NP, D // 2, PW), U32),
            pltpu.VMEM((NP, PW // 2, D), U32),
            pltpu.VMEM((S, D), BF16),
            pltpu.SemaphoreType.DMA((7,)),
            pltpu.SemaphoreType.DMA((4 * n_groups,)),
            pltpu.SemaphoreType.DMA((n_out + 1,)),
        ],
        compiler_params=pltpu.CompilerParams(vmem_limit_bytes=112 * 1024 * 1024),
    )(
        A_x.reshape(S, D), A_wqkv, A_wo, B_x.reshape(S, D), B_mem0.reshape(M, D),
        heads_major(B_Wq), heads_major(B_Wk), heads_major(B_Wv), B_Wo.reshape(HD, D),
    )
    return out.reshape(1, S, 2 * D)
```

```python
import contextlib
import functools

import jax
import jax.numpy as jnp
from jax import lax
import jax.experimental.pallas as pl
import jax.experimental.pallas.tpu as pltpu

BF16 = jnp.bfloat16
F32 = jnp.float32
U32 = jnp.uint32

_NN = (((1,), (0,)), ((), ()))
_NT = (((1,), (1,)), ((), ()))

LANES = 128
NEG = -1000000000.0

A_HEADS = 32
A_WIN = 8
A_DIL = 2
A_HALO = 16
A_ROWS = 128
B_EARLY = 8
A_GROUP = 8


_SCOPES = False


def _scope(name):
    return jax.named_scope(name) if _SCOPES else contextlib.nullcontext()


def _dot(a, b, dn=_NN):
    return lax.dot_general(a, b, dn, preferred_element_type=F32)


def _pack(x):
    return pltpu.bitcast(x, U32)


def _unpack(x):
    return pltpu.bitcast(x, BF16)


def _kernel(
    xa_hbm, wqkv_hbm, woa_hbm, xb_hbm, mem_hbm, wq_hbm, wk_hbm, wv_hbm, wo_hbm,
    out_hbm,
    xa_v, wqkv_raw, woa_raw, perm_v, wqkv_p, woa_p, set_e, set_o, oa_v, outa_v,
    xb_v, mem_v, wq_raw, wk_raw, wv_raw, wo_raw, wq_p, wk_p, wv_p, wo_p,
    xq_v, early_q, outb_v,
    sem_a, sem_w, sem_o,
    *, seg, head_dim,
):
    S, D = xa_v.shape
    M = mem_v.shape[0]
    L = M + seg
    PW = 2 * head_dim
    NP = wq_p.shape[0]
    E = B_EARLY
    n_seg = S // seg
    NT = D // LANES
    R = A_ROWS
    n_it = S // (2 * R)

    qkv_copies = [
        pltpu.make_async_copy(
            wqkv_hbm.at[:, pl.ds(i * D, D)], wqkv_raw.at[i], sem_a.at[i])
        for i in range(3)
    ]
    xa0_copy = pltpu.make_async_copy(
        xa_hbm.at[pl.ds(0, 2 * R)], xa_v.at[pl.ds(0, 2 * R)], sem_a.at[3])
    woa_copy = pltpu.make_async_copy(woa_hbm, woa_raw, sem_a.at[4])
    xa1_copy = pltpu.make_async_copy(
        xa_hbm.at[pl.ds(2 * R, S - 2 * R)], xa_v.at[pl.ds(2 * R, S - 2 * R)], sem_a.at[5])
    xb_copy = pltpu.make_async_copy(xb_hbm, xb_v, sem_a.at[6])
    mem_copy = pltpu.make_async_copy(mem_hbm, mem_v, sem_a.at[7])

    def w_copies(j):
        rows = pl.ds(pl.multiple_of(j * PW, PW), PW)
        return [
            pltpu.make_async_copy(wq_hbm.at[rows], wq_raw.at[rows], sem_w.at[4 * j]),
            pltpu.make_async_copy(wk_hbm.at[rows], wk_raw.at[rows], sem_w.at[4 * j + 1]),
            pltpu.make_async_copy(wv_hbm.at[rows], wv_raw.at[rows], sem_w.at[4 * j + 2]),
            pltpu.make_async_copy(wo_hbm.at[rows], wo_raw.at[rows], sem_w.at[4 * j + 3]),
        ]

    for c in qkv_copies + [xa0_copy, woa_copy, xa1_copy, xb_copy, mem_copy]:
        c.start(priority=1)

    def start_weights(j, carry):
        for c in w_copies(j):
            c.start(priority=1)
        return carry

    lax.fori_loop(0, NP, start_weights, 0)

    dh = D // A_HEADS

    def permute_rows(w):
        w = w.astype(F32)
        for t in range(NT):
            perm_v[t] = w[:, t * LANES:(t + 1) * LANES]
        cols = [
            jnp.concatenate(
                [perm_v[t, pl.ds(d, A_HEADS, stride=dh), :] for d in range(dh)], axis=0)
            for t in range(NT)
        ]
        return _pack(jnp.concatenate(cols, axis=1).astype(BF16))

    for i in range(3):
        with _scope(f"perm{i}"):
            qkv_copies[i].wait()
            wqkv_p[i * D // 2:(i + 1) * D // 2, :] = permute_rows(wqkv_raw[i].T)

    a_scale = dh ** -0.5

    def a_proj(c, dst):
        x = xa_v[pl.ds(pl.multiple_of(c * R, R), R), :]
        qkv = _dot(x, _unpack(wqkv_p[...]), _NT)
        for t in range(3 * NT):
            dst[t, A_HALO:, :] = qkv[:, t * LANES:(t + 1) * LANES]

    def a_halo(src, dst):
        for t in range(NT, 3 * NT):
            dst[t, :A_HALO, :] = src[t, R:, :]

    def a_attn(c, src, first):
        G = A_GROUP

        def scores(g):
            top = A_HALO + g * G
            q = [src[t, top:top + G, :] for t in range(NT)]
            out = []
            for w in range(A_WIN):
                lo = top - A_DIL * w
                s = q[0] * src[NT, lo:lo + G, :]
                for t in range(1, NT):
                    s = s + q[t] * src[NT + t, lo:lo + G, :]
                out.append(s + pltpu.roll(s, 2 * A_HEADS, 1))
            return out

        def fold(g, part):
            out = []
            for w, s in enumerate(part):
                s = (s + pltpu.roll(s, A_HEADS, 1)) * a_scale
                if first and g * G < A_DIL * w:
                    row = g * G + lax.broadcasted_iota(jnp.int32, (G, LANES), 0)
                    s = jnp.where(row >= A_DIL * w, s, NEG)
                out.append(s)
            return out

        def softmax(logits):
            mx = functools.reduce(jnp.maximum, logits)
            e = [jnp.exp(s - mx) for s in logits]
            inv = 1.0 / functools.reduce(jnp.add, e)
            return [x * inv for x in e]

        def values(g, p):
            top = A_HALO + g * G
            o = []
            for t in range(NT):
                acc = p[0] * src[2 * NT + t, top:top + G, :]
                for w in range(1, A_WIN):
                    lo = top - A_DIL * w
                    acc = acc + p[w] * src[2 * NT + t, lo:lo + G, :]
                o.append(acc)
            return jnp.concatenate(o, axis=1)

        n = R // G
        per = max(1, 16 // G)
        st = {}
        for u in range(n + 3):
            if u < n:
                st[u] = scores(u)
            if 0 <= u - 1 < n:
                st[u - 1] = fold(u - 1, st[u - 1])
            if 0 <= u - 2 < n:
                st[u - 2] = softmax(st[u - 2])
            g = u - 3
            if 0 <= g < n:
                st[g] = values(g, st[g])
                if g % per == per - 1:
                    g0 = g - per + 1
                    oa_v[pl.ds(pl.multiple_of(c * R + g0 * G, per * G), per * G), :] = (
                        jnp.concatenate([st[i] for i in range(g0, g + 1)], axis=0).astype(BF16))

    def a_out(c):
        rows = pl.ds(pl.multiple_of(c * 2 * R, 2 * R), 2 * R)
        outa_v[rows, :] = _dot(oa_v[rows, :], _unpack(woa_p[...])).astype(BF16)

    with _scope("a_it0"):
        xa0_copy.wait()
        a_proj(0, set_e)
        for t in range(NT, 3 * NT):
            set_e[t, :A_HALO, :] = jnp.broadcast_to(
                set_e[t, A_HALO:A_HALO + 1, :], (A_HALO, LANES))
        a_halo(set_e, set_o)
        a_attn(0, set_e, True)
        a_proj(1, set_o)

    with _scope("perm3"):
        woa_copy.wait()
        woa_p[...] = permute_rows(woa_raw[...])
        xa1_copy.wait()

    def a_loop(i, carry):
        with _scope("a_it"):
            a_halo(set_o, set_e)
            a_attn(2 * i - 1, set_o, False)
            a_proj(2 * i, set_e)
            a_halo(set_e, set_o)
            a_attn(2 * i, set_e, False)
            a_proj(2 * i + 1, set_o)
        return carry

    lax.fori_loop(1, n_it, a_loop, 0)
    with _scope("a_end"):
        xb_copy.wait()
        mem_copy.wait()
        a_attn(2 * n_it - 1, set_o, False)
        for s in range(n_seg):
            xq_v[s * E:(s + 1) * E, :] = xb_v[(s + 1) * seg - E:(s + 1) * seg, :].astype(F32)

    ppi = NP // n_it

    def b_prep(i, carry):
        with _scope("b_prep"):
            for jj in range(ppi):
                for c in w_copies(i * ppi + jj):
                    c.wait()
            a_out(i)
            rows = pl.ds(pl.multiple_of(i * ppi * PW, PW), PW)
            early_q[i] = _dot(xq_v[...], wq_raw[rows, :], _NT)
            for jj in range(ppi):
                j = i * ppi + jj
                rows = pl.ds(pl.multiple_of(j * PW, PW), PW)
                wq_p[j] = _pack(wq_raw[rows, :].T)
                wk_p[j] = _pack(wk_raw[rows, :].T)
                wv_p[j] = _pack(wv_raw[rows, :].T)
                wo_p[j] = _pack(wo_raw[rows, :])
        return carry

    lax.fori_loop(0, n_it, b_prep, 0)

    outa_copy = pltpu.make_async_copy(outa_v, out_hbm.at[:, pl.ds(0, D)], sem_o.at[0])
    outa_copy.start()

    b_scale = head_dim ** -0.5

    order = []
    for t in range(NP):
        order.append(("q", t))
        order.append(("k", t))
        order.append(("v", t))
        if t >= 1:
            order.append(("pv", t - 1))
        order.append(("s", t))
        if t >= 5:
            order.append(("o", t - 5))
    order += [("o", NP - 5), ("o", NP - 4), ("o", NP - 3), ("pv", NP - 1),
              ("o", NP - 2), ("o", NP - 1)]

    def b_step(s, mem):
        r0 = pl.multiple_of(s * seg, seg)
        h = jnp.concatenate([mem, xb_v[pl.ds(r0, seg), :].astype(F32)], axis=0)
        lane = lax.broadcasted_iota(jnp.int32, (L, LANES), 1)
        row = lax.broadcasted_iota(jnp.int32, (L, LANES), 0)
        is_a = lane < L
        is_b = (lane >= L) & (lane < 2 * L)
        visible = (row < M) | (row >= jnp.where(is_a, lane, lane - L))
        feat_a = lax.broadcasted_iota(jnp.int32, (L, PW), 1) < head_dim

        def block_diag(t):
            return jnp.concatenate(
                [jnp.where(feat_a, t, 0.0), jnp.where(feat_a, 0.0, t),
                 jnp.zeros((LANES - 2 * L, PW), F32)], axis=0).astype(BF16)

        q, k, v, p, o = {}, {}, {}, {}, {}
        acc = None
        for op, j in order:
            if op == "q":
                if j % ppi == 0:
                    q[j] = jnp.concatenate(
                        [_dot(h[:L - E], _unpack(wq_p[j])),
                         early_q[j // ppi, pl.ds(pl.multiple_of(s * E, E), E), :]], axis=0)
                else:
                    q[j] = _dot(h, _unpack(wq_p[j]))
            elif op == "k":
                k[j] = _dot(h, _unpack(wk_p[j]))
            elif op == "v":
                v[j] = _dot(h, _unpack(wv_p[j]))
            elif op == "s":
                sc = _dot(q[j], block_diag(k[j]), _NT) * b_scale
                sc = jnp.where(visible, sc, NEG)
                m_a = jnp.max(jnp.where(is_a, sc, -jnp.inf), axis=1, keepdims=True)
                m_b = jnp.max(jnp.where(is_b, sc, -jnp.inf), axis=1, keepdims=True)
                e = jnp.exp(sc - jnp.where(is_a, m_a, m_b))
                e_a = jnp.where(is_a, e, 0.0)
                e_b = jnp.where(is_b, e, 0.0)
                l_a = jnp.sum(e_a, axis=1, keepdims=True)
                l_b = jnp.sum(e_b, axis=1, keepdims=True)
                p[j] = (e_a + e_b) / jnp.where(is_a, l_a, l_b)
            elif op == "pv":
                o[j] = _dot(p[j], block_diag(v[j]))
            else:
                d = _dot(o[j], _unpack(wo_p[j]))
                acc = d if acc is None else acc + d
        outb_v[pl.ds(r0, seg), :] = acc[M:].astype(BF16)
        return acc[:M]

    n_out = sem_o.shape[0] - 1
    spo = n_seg // n_out

    def outb_copy(i):
        rows = pl.ds(pl.multiple_of(i * spo * seg, spo * seg), spo * seg)
        return pltpu.make_async_copy(
            outb_v.at[rows], out_hbm.at[rows, pl.ds(D, D)], sem_o.at[i + 1])

    def b_outer(i, mem):
        with _scope("b_outer"):
            mem = lax.fori_loop(i * spo, (i + 1) * spo, b_step, mem)
        outb_copy(i).start()
        return mem

    lax.fori_loop(0, n_out, b_outer, mem_v[...].astype(F32))

    outa_copy.wait()
    for i in range(n_out):
        outb_copy(i).wait()


@functools.partial(jax.jit, static_argnames=("B_seg_len",))
def pallas_concat_heads__sliding_local_dilated__memory_aug_recurrent_mem_tr__prompt_kernel(
    A_x: jax.Array,
    A_wqkv: jax.Array,
    A_wo: jax.Array,
    B_x: jax.Array,
    B_mem0: jax.Array,
    B_Wq: jax.Array,
    B_Wk: jax.Array,
    B_Wv: jax.Array,
    B_Wo: jax.Array,
    B_seg_len: int,
):
    _, S, D = A_x.shape
    _, H, Dh = B_Wq.shape
    M = B_mem0.shape[1]
    HD = H * Dh
    NP = H // 2
    PW = 2 * Dh
    n_early = S // B_seg_len * B_EARLY
    n_out = 8

    def heads_major(w):
        return w.transpose(1, 2, 0).reshape(HD, D)

    qkv_set = pltpu.VMEM((3 * D // LANES, A_HALO + A_ROWS, LANES), F32)
    out = pl.pallas_call(
        functools.partial(_kernel, seg=B_seg_len, head_dim=Dh),
        out_shape=jax.ShapeDtypeStruct((S, 2 * D), BF16),
        in_specs=[pl.BlockSpec(memory_space=pltpu.HBM)] * 9,
        out_specs=pl.BlockSpec(memory_space=pltpu.HBM),
        scratch_shapes=[
            pltpu.VMEM((S, D), BF16),
            pltpu.VMEM((3, D, D), BF16),
            pltpu.VMEM((D, D), BF16),
            pltpu.VMEM((D // LANES, D, LANES), F32),
            pltpu.VMEM((3 * D // 2, D), U32),
            pltpu.VMEM((D // 2, D), U32),
            qkv_set,
            qkv_set,
            pltpu.VMEM((S, D), BF16),
            pltpu.VMEM((S, D), BF16),
            pltpu.VMEM((S, D), BF16),
            pltpu.VMEM((M, D), BF16),
            pltpu.VMEM((HD, D), BF16),
            pltpu.VMEM((HD, D), BF16),
            pltpu.VMEM((HD, D), BF16),
            pltpu.VMEM((HD, D), BF16),
            pltpu.VMEM((NP, D // 2, PW), U32),
            pltpu.VMEM((NP, D // 2, PW), U32),
            pltpu.VMEM((NP, D // 2, PW), U32),
            pltpu.VMEM((NP, PW // 2, D), U32),
            pltpu.VMEM((n_early, D), F32),
            pltpu.VMEM((S // (2 * A_ROWS), n_early, PW), F32),
            pltpu.VMEM((S, D), BF16),
            pltpu.SemaphoreType.DMA((8,)),
            pltpu.SemaphoreType.DMA((4 * NP,)),
            pltpu.SemaphoreType.DMA((n_out + 1,)),
        ],
        compiler_params=pltpu.CompilerParams(vmem_limit_bytes=120 * 1024 * 1024),
    )(
        A_x.reshape(S, D), A_wqkv, A_wo, B_x.reshape(S, D), B_mem0.reshape(M, D),
        heads_major(B_Wq), heads_major(B_Wk), heads_major(B_Wv), B_Wo.reshape(HD, D),
    )
    return out.reshape(1, S, 2 * D)
```

```python
import contextlib
import functools

import jax
import jax.numpy as jnp
from jax import lax
import jax.experimental.pallas as pl
import jax.experimental.pallas.tpu as pltpu

BF16 = jnp.bfloat16
F32 = jnp.float32
U32 = jnp.uint32

_NN = (((1,), (0,)), ((), ()))
_NT = (((1,), (1,)), ((), ()))

LANES = 128
NEG = -1000000000.0

A_HEADS = 32
A_WIN = 8
A_DIL = 2
A_HALO = 16
A_ROWS = 128
B_EARLY = 8
B_UNROLL = 4
A_GROUP = 8


_SCOPES = False


def _scope(name):
    return jax.named_scope(name) if _SCOPES else contextlib.nullcontext()


def _dot(a, b, dn=_NN):
    return lax.dot_general(a, b, dn, preferred_element_type=F32)


def _pack(x):
    return pltpu.bitcast(x, U32)


def _unpack(x):
    return pltpu.bitcast(x, BF16)


B_ORDER = ("kqvpso", 5, 1, 0, 3)


def _b_order(n):
    pattern, lag_o, lag_p, lag_s, n_before = B_ORDER
    lag = dict(q=0, k=0, v=0, s=lag_s, p=lag_p, o=lag_o)
    order = []
    for t in range(n):
        for op in pattern:
            if t - lag[op] >= 0:
                order.append((op, t - lag[op]))
    rest_o = [("o", j) for j in range(n - lag_o, n)]
    for j in range(n - lag_s, n):
        order.append(rest_o.pop(0))
        order.append(("s", j))
    for j in range(n - lag_p, n - 1):
        order.append(rest_o.pop(0))
        order.append(("p", j))
    order += rest_o[:n_before] + [("p", n - 1)] + rest_o[n_before:]
    return order


def _kernel(
    xa_hbm, wqkv_hbm, woa_hbm, xb_hbm, mem_hbm, wq_hbm, wk_hbm, wv_hbm, wo_hbm,
    out_hbm,
    xa_v, wqkv_raw, woa_raw, perm_v, wqkv_p, woa_p, set_e, set_o, oa_v, outa_v,
    xb_v, mem_v, wq_raw, wk_raw, wv_raw, wo_raw, wq_p, wk_p, wv_p, wo_p,
    xq_v, early_q, outb_v,
    sem_a, sem_w, sem_o,
    *, seg, head_dim,
):
    S, D = xa_v.shape
    M = mem_v.shape[0]
    L = M + seg
    PW = 2 * head_dim
    NP = wq_p.shape[0]
    E = B_EARLY
    n_seg = S // seg
    NT = D // LANES
    R = A_ROWS
    n_it = S // (2 * R)

    qkv_copies = [
        pltpu.make_async_copy(
            wqkv_hbm.at[:, pl.ds(i * D, D)], wqkv_raw.at[i], sem_a.at[i])
        for i in range(3)
    ]
    xa0_copy = pltpu.make_async_copy(
        xa_hbm.at[pl.ds(0, 2 * R)], xa_v.at[pl.ds(0, 2 * R)], sem_a.at[3])
    woa_copy = pltpu.make_async_copy(woa_hbm, woa_raw, sem_a.at[4])
    xa1_copy = pltpu.make_async_copy(
        xa_hbm.at[pl.ds(2 * R, S - 2 * R)], xa_v.at[pl.ds(2 * R, S - 2 * R)], sem_a.at[5])
    xb_copy = pltpu.make_async_copy(xb_hbm, xb_v, sem_a.at[6])
    mem_copy = pltpu.make_async_copy(mem_hbm, mem_v, sem_a.at[7])

    def w_copies(j):
        rows = pl.ds(pl.multiple_of(j * PW, PW), PW)
        return [
            pltpu.make_async_copy(wq_hbm.at[rows], wq_raw.at[rows], sem_w.at[4 * j]),
            pltpu.make_async_copy(wk_hbm.at[rows], wk_raw.at[rows], sem_w.at[4 * j + 1]),
            pltpu.make_async_copy(wv_hbm.at[rows], wv_raw.at[rows], sem_w.at[4 * j + 2]),
            pltpu.make_async_copy(wo_hbm.at[rows], wo_raw.at[rows], sem_w.at[4 * j + 3]),
        ]

    for c in qkv_copies + [xa0_copy, woa_copy, xa1_copy, xb_copy, mem_copy]:
        c.start(priority=1)

    def start_weights(j, carry):
        for c in w_copies(j):
            c.start(priority=1)
        return carry

    lax.fori_loop(0, NP, start_weights, 0)

    dh = D // A_HEADS

    def permute_rows(w):
        w = w.astype(F32)
        for t in range(NT):
            perm_v[t] = w[:, t * LANES:(t + 1) * LANES]
        cols = [
            jnp.concatenate(
                [perm_v[t, pl.ds(d, A_HEADS, stride=dh), :] for d in range(dh)], axis=0)
            for t in range(NT)
        ]
        return _pack(jnp.concatenate(cols, axis=1).astype(BF16))

    for i in range(3):
        with _scope(f"perm{i}"):
            qkv_copies[i].wait()
            wqkv_p[i * D // 2:(i + 1) * D // 2, :] = permute_rows(wqkv_raw[i].T)

    a_scale = dh ** -0.5

    def a_proj(c, dst):
        x = xa_v[pl.ds(pl.multiple_of(c * R, R), R), :]
        qkv = _dot(x, _unpack(wqkv_p[...]), _NT)
        for t in range(3 * NT):
            dst[t, A_HALO:, :] = qkv[:, t * LANES:(t + 1) * LANES]

    def a_halo(src, dst):
        for t in range(NT, 3 * NT):
            dst[t, :A_HALO, :] = src[t, R:, :]

    def a_attn(c, src, first):
        G = A_GROUP

        def scores(g):
            top = A_HALO + g * G
            q = [src[t, top:top + G, :] for t in range(NT)]
            out = []
            for w in range(A_WIN):
                lo = top - A_DIL * w
                s = q[0] * src[NT, lo:lo + G, :]
                for t in range(1, NT):
                    s = s + q[t] * src[NT + t, lo:lo + G, :]
                out.append(s + pltpu.roll(s, 2 * A_HEADS, 1))
            return out

        def fold(g, part):
            out = []
            for w, s in enumerate(part):
                s = (s + pltpu.roll(s, A_HEADS, 1)) * a_scale
                if first and g * G < A_DIL * w:
                    row = g * G + lax.broadcasted_iota(jnp.int32, (G, LANES), 0)
                    s = jnp.where(row >= A_DIL * w, s, NEG)
                out.append(s)
            return out

        def softmax(logits):
            mx = functools.reduce(jnp.maximum, logits)
            e = [jnp.exp(s - mx) for s in logits]
            inv = 1.0 / functools.reduce(jnp.add, e)
            return [x * inv for x in e]

        def values(g, p):
            top = A_HALO + g * G
            o = []
            for t in range(NT):
                acc = p[0] * src[2 * NT + t, top:top + G, :]
                for w in range(1, A_WIN):
                    lo = top - A_DIL * w
                    acc = acc + p[w] * src[2 * NT + t, lo:lo + G, :]
                o.append(acc)
            return jnp.concatenate(o, axis=1)

        n = R // G
        per = max(1, 16 // G)
        st = {}
        for u in range(n + 3):
            if u < n:
                st[u] = scores(u)
            if 0 <= u - 1 < n:
                st[u - 1] = fold(u - 1, st[u - 1])
            if 0 <= u - 2 < n:
                st[u - 2] = softmax(st[u - 2])
            g = u - 3
            if 0 <= g < n:
                st[g] = values(g, st[g])
                if g % per == per - 1:
                    g0 = g - per + 1
                    oa_v[pl.ds(pl.multiple_of(c * R + g0 * G, per * G), per * G), :] = (
                        jnp.concatenate([st[i] for i in range(g0, g + 1)], axis=0).astype(BF16))

    def a_out(c):
        rows = pl.ds(pl.multiple_of(c * 2 * R, 2 * R), 2 * R)
        outa_v[rows, :] = _dot(oa_v[rows, :], _unpack(woa_p[...])).astype(BF16)

    with _scope("a_it0"):
        xa0_copy.wait()
        a_proj(0, set_e)
        for t in range(NT, 3 * NT):
            set_e[t, :A_HALO, :] = jnp.broadcast_to(
                set_e[t, A_HALO:A_HALO + 1, :], (A_HALO, LANES))
        a_halo(set_e, set_o)
        a_attn(0, set_e, True)
        a_proj(1, set_o)

    with _scope("perm3"):
        woa_copy.wait()
        woa_p[...] = permute_rows(woa_raw[...])
        xa1_copy.wait()

    def a_loop(i, carry):
        with _scope("a_it"):
            a_halo(set_o, set_e)
            a_attn(2 * i - 1, set_o, False)
            a_proj(2 * i, set_e)
            a_halo(set_e, set_o)
            a_attn(2 * i, set_e, False)
            a_proj(2 * i + 1, set_o)
        return carry

    lax.fori_loop(1, n_it, a_loop, 0)
    with _scope("a_end"):
        xb_copy.wait()
        mem_copy.wait()
        a_attn(2 * n_it - 1, set_o, False)
        for s in range(n_seg):
            xq_v[s * E:(s + 1) * E, :] = xb_v[(s + 1) * seg - E:(s + 1) * seg, :].astype(F32)

    ppi = NP // n_it

    def b_prep(i, carry):
        with _scope("b_prep"):
            for jj in range(ppi):
                for c in w_copies(i * ppi + jj):
                    c.wait()
            a_out(i)
            rows = pl.ds(pl.multiple_of(i * ppi * PW, PW), PW)
            early_q[i] = _dot(xq_v[...], wq_raw[rows, :], _NT)
            for jj in range(ppi):
                j = i * ppi + jj
                rows = pl.ds(pl.multiple_of(j * PW, PW), PW)
                wq_p[j] = _pack(wq_raw[rows, :].T)
                wk_p[j] = _pack(wk_raw[rows, :].T)
                wv_p[j] = _pack(wv_raw[rows, :].T)
                wo_p[j] = _pack(wo_raw[rows, :])
        return carry

    lax.fori_loop(0, n_it, b_prep, 0)

    outa_copy = pltpu.make_async_copy(outa_v, out_hbm.at[:, pl.ds(0, D)], sem_o.at[0])
    outa_copy.start()

    b_scale = head_dim ** -0.5

    order = _b_order(NP)

    def b_step(s, mem):
        r0 = pl.multiple_of(s * seg, seg)
        h = jnp.concatenate([mem, xb_v[pl.ds(r0, seg), :].astype(F32)], axis=0)
        lane = lax.broadcasted_iota(jnp.int32, (L, LANES), 1)
        row = lax.broadcasted_iota(jnp.int32, (L, LANES), 0)
        is_a = lane < L
        is_b = (lane >= L) & (lane < 2 * L)
        visible = (row < M) | (row >= jnp.where(is_a, lane, lane - L))
        feat_a = lax.broadcasted_iota(jnp.int32, (L, PW), 1) < head_dim

        def block_diag(t):
            return jnp.concatenate(
                [jnp.where(feat_a, t, 0.0), jnp.where(feat_a, 0.0, t),
                 jnp.zeros((LANES - 2 * L, PW), F32)], axis=0).astype(BF16)

        q, k, v, p, o = {}, {}, {}, {}, {}
        acc = None
        for op, j in order:
            if op == "q":
                if j % ppi == 0:
                    q[j] = jnp.concatenate(
                        [_dot(h[:L - E], _unpack(wq_p[j])),
                         early_q[j // ppi, pl.ds(pl.multiple_of(s * E, E), E), :]], axis=0)
                else:
                    q[j] = _dot(h, _unpack(wq_p[j]))
            elif op == "k":
                k[j] = _dot(h, _unpack(wk_p[j]))
            elif op == "v":
                v[j] = _dot(h, _unpack(wv_p[j]))
            elif op == "s":
                sc = _dot(q[j], block_diag(k[j]), _NT) * b_scale
                sc = jnp.where(visible, sc, NEG)
                m_a = jnp.max(jnp.where(is_a, sc, -jnp.inf), axis=1, keepdims=True)
                m_b = jnp.max(jnp.where(is_b, sc, -jnp.inf), axis=1, keepdims=True)
                e = jnp.exp(sc - jnp.where(is_a, m_a, m_b))
                e_a = jnp.where(is_a, e, 0.0)
                e_b = jnp.where(is_b, e, 0.0)
                l_a = jnp.sum(e_a, axis=1, keepdims=True)
                l_b = jnp.sum(e_b, axis=1, keepdims=True)
                p[j] = (e_a + e_b) / jnp.where(is_a, l_a, l_b)
            elif op == "p":
                o[j] = _dot(p[j], block_diag(v[j]))
            else:
                d = _dot(o[j], _unpack(wo_p[j]))
                acc = d if acc is None else acc + d
        outb_v[pl.ds(r0, seg), :] = acc[M:].astype(BF16)
        return acc[:M]

    n_out = sem_o.shape[0] - 1
    spo = n_seg // n_out

    def outb_copy(i):
        rows = pl.ds(pl.multiple_of(i * spo * seg, spo * seg), spo * seg)
        return pltpu.make_async_copy(
            outb_v.at[rows], out_hbm.at[rows, pl.ds(D, D)], sem_o.at[i + 1])

    def b_outer(i, mem):
        with _scope("b_outer"):
            mem = lax.fori_loop(0, spo, lambda u, m: b_step(i * spo + u, m), mem, unroll=B_UNROLL)
        outb_copy(i).start()
        return mem

    lax.fori_loop(0, n_out, b_outer, mem_v[...].astype(F32))

    outa_copy.wait()
    for i in range(n_out):
        outb_copy(i).wait()


@functools.partial(jax.jit, static_argnames=("B_seg_len",))
def pallas_concat_heads__sliding_local_dilated__memory_aug_recurrent_mem_tr__prompt_kernel(
    A_x: jax.Array,
    A_wqkv: jax.Array,
    A_wo: jax.Array,
    B_x: jax.Array,
    B_mem0: jax.Array,
    B_Wq: jax.Array,
    B_Wk: jax.Array,
    B_Wv: jax.Array,
    B_Wo: jax.Array,
    B_seg_len: int,
):
    _, S, D = A_x.shape
    _, H, Dh = B_Wq.shape
    M = B_mem0.shape[1]
    HD = H * Dh
    NP = H // 2
    PW = 2 * Dh
    n_early = S // B_seg_len * B_EARLY
    n_out = 8

    def heads_major(w):
        return w.transpose(1, 2, 0).reshape(HD, D)

    qkv_set = pltpu.VMEM((3 * D // LANES, A_HALO + A_ROWS, LANES), F32)
    out = pl.pallas_call(
        functools.partial(_kernel, seg=B_seg_len, head_dim=Dh),
        out_shape=jax.ShapeDtypeStruct((S, 2 * D), BF16),
        in_specs=[pl.BlockSpec(memory_space=pltpu.HBM)] * 9,
        out_specs=pl.BlockSpec(memory_space=pltpu.HBM),
        scratch_shapes=[
            pltpu.VMEM((S, D), BF16),
            pltpu.VMEM((3, D, D), BF16),
            pltpu.VMEM((D, D), BF16),
            pltpu.VMEM((D // LANES, D, LANES), F32),
            pltpu.VMEM((3 * D // 2, D), U32),
            pltpu.VMEM((D // 2, D), U32),
            qkv_set,
            qkv_set,
            pltpu.VMEM((S, D), BF16),
            pltpu.VMEM((S, D), BF16),
            pltpu.VMEM((S, D), BF16),
            pltpu.VMEM((M, D), BF16),
            pltpu.VMEM((HD, D), BF16),
            pltpu.VMEM((HD, D), BF16),
            pltpu.VMEM((HD, D), BF16),
            pltpu.VMEM((HD, D), BF16),
            pltpu.VMEM((NP, D // 2, PW), U32),
            pltpu.VMEM((NP, D // 2, PW), U32),
            pltpu.VMEM((NP, D // 2, PW), U32),
            pltpu.VMEM((NP, PW // 2, D), U32),
            pltpu.VMEM((n_early, D), F32),
            pltpu.VMEM((S // (2 * A_ROWS), n_early, PW), F32),
            pltpu.VMEM((S, D), BF16),
            pltpu.SemaphoreType.DMA((8,)),
            pltpu.SemaphoreType.DMA((4 * NP,)),
            pltpu.SemaphoreType.DMA((n_out + 1,)),
        ],
        compiler_params=pltpu.CompilerParams(vmem_limit_bytes=120 * 1024 * 1024),
    )(
        A_x.reshape(S, D), A_wqkv, A_wo, B_x.reshape(S, D), B_mem0.reshape(M, D),
        heads_major(B_Wq), heads_major(B_Wk), heads_major(B_Wv), B_Wo.reshape(HD, D),
    )
    return out.reshape(1, S, 2 * D)
```

```python
import contextlib
import functools

import jax
import jax.numpy as jnp
from jax import lax
import jax.experimental.pallas as pl
import jax.experimental.pallas.tpu as pltpu

BF16 = jnp.bfloat16
F32 = jnp.float32
U32 = jnp.uint32

_NN = (((1,), (0,)), ((), ()))
_NT = (((1,), (1,)), ((), ()))

LANES = 128
NEG = -1000000000.0

A_HEADS = 32
A_WIN = 8
A_DIL = 2
A_HALO = 16
A_ROWS = 128
B_EARLY = 8
B_UNROLL = 4
A_SLOTS = 2
A_GROUP = 8


_SCOPES = False


def _scope(name):
    return jax.named_scope(name) if _SCOPES else contextlib.nullcontext()


def _dot(a, b, dn=_NN):
    return lax.dot_general(a, b, dn, preferred_element_type=F32)


def _pack(x):
    return pltpu.bitcast(x, U32)


def _unpack(x):
    return pltpu.bitcast(x, BF16)


B_ORDER = ("kqvpso", 5, 1, 0, 3)


def _b_order(n):
    pattern, lag_o, lag_p, lag_s, n_before = B_ORDER
    lag = dict(q=0, k=0, v=0, s=lag_s, p=lag_p, o=lag_o)
    order = []
    for t in range(n):
        for op in pattern:
            if t - lag[op] >= 0:
                order.append((op, t - lag[op]))
    rest_o = [("o", j) for j in range(n - lag_o, n)]
    for j in range(n - lag_s, n):
        order.append(rest_o.pop(0))
        order.append(("s", j))
    for j in range(n - lag_p, n - 1):
        order.append(rest_o.pop(0))
        order.append(("p", j))
    order += rest_o[:n_before] + [("p", n - 1)] + rest_o[n_before:]
    return order


def _kernel(
    xa_hbm, wqkv_hbm, woa_hbm, xb_hbm, mem_hbm, wq_hbm, wk_hbm, wv_hbm, wo_hbm,
    out_hbm,
    xa_v, wqkv_raw, woa_raw, perm_v, wqkv_p, woa_p, set_e, set_o, slot_v, oa_v,
    xb_v, mem_v, wq_raw, wk_raw, wv_raw, wo_raw, wq_p, wk_p, wv_p, wo_p,
    xq_v, early_q, out_v,
    sem_a, sem_w, sem_o,
    *, seg, head_dim,
):
    S, D = xa_v.shape
    M = mem_v.shape[0]
    L = M + seg
    PW = 2 * head_dim
    NP = wq_p.shape[0]
    E = B_EARLY
    n_seg = S // seg
    NT = D // LANES
    R = A_ROWS
    n_it = S // (2 * R)

    qkv_copies = [
        pltpu.make_async_copy(
            wqkv_hbm.at[:, pl.ds(i * D, D)], wqkv_raw.at[i], sem_a.at[i])
        for i in range(3)
    ]
    xa0_copy = pltpu.make_async_copy(
        xa_hbm.at[pl.ds(0, 2 * R)], xa_v.at[pl.ds(0, 2 * R)], sem_a.at[3])
    woa_copy = pltpu.make_async_copy(woa_hbm, woa_raw, sem_a.at[4])
    xa1_copy = pltpu.make_async_copy(
        xa_hbm.at[pl.ds(2 * R, S - 2 * R)], xa_v.at[pl.ds(2 * R, S - 2 * R)], sem_a.at[5])
    xb_copy = pltpu.make_async_copy(xb_hbm, xb_v, sem_a.at[6])
    mem_copy = pltpu.make_async_copy(mem_hbm, mem_v, sem_a.at[7])

    def w_copies(j):
        rows = pl.ds(pl.multiple_of(j * PW, PW), PW)
        return [
            pltpu.make_async_copy(wq_hbm.at[rows], wq_raw.at[rows], sem_w.at[4 * j]),
            pltpu.make_async_copy(wk_hbm.at[rows], wk_raw.at[rows], sem_w.at[4 * j + 1]),
            pltpu.make_async_copy(wv_hbm.at[rows], wv_raw.at[rows], sem_w.at[4 * j + 2]),
            pltpu.make_async_copy(wo_hbm.at[rows], wo_raw.at[rows], sem_w.at[4 * j + 3]),
        ]

    for c in qkv_copies + [xa0_copy, xa1_copy, woa_copy, xb_copy, mem_copy]:
        c.start(priority=1)

    def start_weights(j, carry):
        for c in w_copies(j):
            c.start(priority=1)
        return carry

    lax.fori_loop(0, NP, start_weights, 0)

    dh = D // A_HEADS

    def permute_rows(w):
        w = w.astype(F32)
        for t in range(NT):
            perm_v[t] = w[:, t * LANES:(t + 1) * LANES]
        cols = [
            jnp.concatenate(
                [perm_v[t, pl.ds(d, A_HEADS, stride=dh), :] for d in range(dh)], axis=0)
            for t in range(NT)
        ]
        return _pack(jnp.concatenate(cols, axis=1).astype(BF16))

    for i in range(3):
        with _scope(f"perm{i}"):
            qkv_copies[i].wait()
            wqkv_p[i * D // 2:(i + 1) * D // 2, :] = permute_rows(wqkv_raw[i].T)

    a_scale = dh ** -0.5

    def a_proj(c, dst):
        x = xa_v[pl.ds(pl.multiple_of(c * R, R), R), :]
        qkv = _dot(x, _unpack(wqkv_p[...]), _NT)
        for t in range(3 * NT):
            dst[t, A_HALO:, :] = qkv[:, t * LANES:(t + 1) * LANES]

    def a_halo(src, dst):
        for t in range(NT, 3 * NT):
            dst[t, :A_HALO, :] = src[t, R:, :]

    def a_attn(c, src, first):
        G = A_GROUP

        def scores(g):
            top = A_HALO + g * G
            for t in range(NT):
                slot_v[g % A_SLOTS, t] = src[t, top:top + G, :]
            q = [slot_v[g % A_SLOTS, t] for t in range(NT)]
            out = []
            for w in range(A_WIN):
                lo = top - A_DIL * w
                s = q[0] * src[NT, lo:lo + G, :]
                for t in range(1, NT):
                    s = s + q[t] * src[NT + t, lo:lo + G, :]
                out.append(s + pltpu.roll(s, 2 * A_HEADS, 1))
            return out

        def fold(g, part):
            out = []
            for w, s in enumerate(part):
                s = (s + pltpu.roll(s, A_HEADS, 1)) * a_scale
                if first and g * G < A_DIL * w:
                    row = g * G + lax.broadcasted_iota(jnp.int32, (G, LANES), 0)
                    s = jnp.where(row >= A_DIL * w, s, NEG)
                out.append(s)
            return out

        def softmax(logits):
            mx = functools.reduce(jnp.maximum, logits)
            e = [jnp.exp(s - mx) for s in logits]
            inv = 1.0 / functools.reduce(jnp.add, e)
            return [x * inv for x in e]

        def values(g, p):
            top = A_HALO + g * G
            for w in range(A_WIN):
                slot_v[g % A_SLOTS, w] = p[w]
            p = [slot_v[g % A_SLOTS, w] for w in range(A_WIN)]
            o = []
            for t in range(NT):
                acc = p[0] * src[2 * NT + t, top:top + G, :]
                for w in range(1, A_WIN):
                    lo = top - A_DIL * w
                    acc = acc + p[w] * src[2 * NT + t, lo:lo + G, :]
                o.append(acc)
            return jnp.concatenate(o, axis=1)

        n = R // G
        per = max(1, 16 // G)
        st = {}
        for u in range(n):
            st[u] = softmax(fold(u, scores(u)))
            g = u
            if 0 <= g < n:
                st[g] = values(g, st[g])
                if g % per == per - 1:
                    g0 = g - per + 1
                    oa_v[pl.ds(pl.multiple_of(c * R + g0 * G, per * G), per * G), :] = (
                        jnp.concatenate([st[i] for i in range(g0, g + 1)], axis=0).astype(BF16))

    with _scope("a_it0"):
        xa0_copy.wait()
        a_proj(0, set_e)
        for t in range(NT, 3 * NT):
            set_e[t, :A_HALO, :] = jnp.broadcast_to(
                set_e[t, A_HALO:A_HALO + 1, :], (A_HALO, LANES))
        a_halo(set_e, set_o)
        a_attn(0, set_e, True)
        a_proj(1, set_o)

    xa1_copy.wait()

    def a_loop(i, carry):
        with _scope("a_it"):
            a_halo(set_o, set_e)
            a_attn(2 * i - 1, set_o, False)
            a_proj(2 * i, set_e)
            a_halo(set_e, set_o)
            a_attn(2 * i, set_e, False)
            a_proj(2 * i + 1, set_o)
        return carry

    lax.fori_loop(1, n_it, a_loop, 0)
    with _scope("a_end"):
        xb_copy.wait()
        mem_copy.wait()
        woa_copy.wait()
        woa_p[...] = permute_rows(woa_raw[...])
        a_attn(2 * n_it - 1, set_o, False)
        for s in range(n_seg):
            xq_v[s * E:(s + 1) * E, :] = xb_v[(s + 1) * seg - E:(s + 1) * seg, :].astype(F32)

    ppi = 2
    n_prep = NP // ppi

    def b_prep(i, carry):
        with _scope("b_prep"):
            for jj in range(ppi):
                for c in w_copies(i * ppi + jj):
                    c.wait()
            for jj in range(ppi):
                j = i * ppi + jj
                rows = pl.ds(pl.multiple_of(j * PW, PW), PW)
                early_q[j] = _dot(xq_v[...], wq_raw[rows, :], _NT)
                wq_p[j] = _pack(wq_raw[rows, :].T)
                wk_p[j] = _pack(wk_raw[rows, :].T)
                wv_p[j] = _pack(wv_raw[rows, :].T)
                wo_p[j] = _pack(wo_raw[rows, :])
        return carry

    lax.fori_loop(0, n_prep, b_prep, 0)

    b_scale = head_dim ** -0.5

    order = _b_order(NP)

    def b_step(s, mem):
        r0 = pl.multiple_of(s * seg, seg)
        h = jnp.concatenate([mem, xb_v[pl.ds(r0, seg), :].astype(F32)], axis=0)
        lane = lax.broadcasted_iota(jnp.int32, (L, LANES), 1)
        row = lax.broadcasted_iota(jnp.int32, (L, LANES), 0)
        is_a = lane < L
        is_b = (lane >= L) & (lane < 2 * L)
        visible = (row < M) | (row >= jnp.where(is_a, lane, lane - L))
        feat_a = lax.broadcasted_iota(jnp.int32, (L, PW), 1) < head_dim

        def block_diag(t):
            return jnp.concatenate(
                [jnp.where(feat_a, t, 0.0), jnp.where(feat_a, 0.0, t),
                 jnp.zeros((LANES - 2 * L, PW), F32)], axis=0).astype(BF16)

        q, k, v, p, o = {}, {}, {}, {}, {}
        acc = None
        for op, j in order:
            if op == "q":
                q[j] = jnp.concatenate(
                    [_dot(h[:L - E], _unpack(wq_p[j])),
                     early_q[j, pl.ds(pl.multiple_of(s * E, E), E), :]], axis=0)
            elif op == "k":
                k[j] = _dot(h, _unpack(wk_p[j]))
            elif op == "v":
                v[j] = _dot(h, _unpack(wv_p[j]))
            elif op == "s":
                sc = _dot(q[j], block_diag(k[j]), _NT) * b_scale
                sc = jnp.where(visible, sc, NEG)
                m_a = jnp.max(jnp.where(is_a, sc, -jnp.inf), axis=1, keepdims=True)
                m_b = jnp.max(jnp.where(is_b, sc, -jnp.inf), axis=1, keepdims=True)
                e = jnp.exp(sc - jnp.where(is_a, m_a, m_b))
                e_a = jnp.where(is_a, e, 0.0)
                e_b = jnp.where(is_b, e, 0.0)
                l_a = jnp.sum(e_a, axis=1, keepdims=True)
                l_b = jnp.sum(e_b, axis=1, keepdims=True)
                p[j] = (e_a + e_b) / jnp.where(is_a, l_a, l_b)
            elif op == "p":
                o[j] = _dot(p[j], block_diag(v[j]))
            else:
                d = _dot(o[j], _unpack(wo_p[j]))
                acc = d if acc is None else acc + d
        out_v[pl.ds(r0, seg), D:] = acc[M:].astype(BF16)
        out_v[pl.ds(r0, seg), :D] = _dot(
            oa_v[pl.ds(r0, seg), :], _unpack(woa_p[...])).astype(BF16)
        return acc[:M]

    n_out = sem_o.shape[0]
    spo = n_seg // n_out

    def outb_copy(i):
        rows = pl.ds(pl.multiple_of(i * spo * seg, spo * seg), spo * seg)
        return pltpu.make_async_copy(
            out_v.at[rows], out_hbm.at[rows], sem_o.at[i])

    def b_outer(i, mem):
        with _scope("b_outer"):
            mem = lax.fori_loop(0, spo, lambda u, m: b_step(i * spo + u, m), mem, unroll=B_UNROLL)
        outb_copy(i).start()
        return mem

    lax.fori_loop(0, n_out, b_outer, mem_v[...].astype(F32))

    for i in range(n_out):
        outb_copy(i).wait()


@functools.partial(jax.jit, static_argnames=("B_seg_len",))
def pallas_concat_heads__sliding_local_dilated__memory_aug_recurrent_mem_tr__prompt_kernel(
    A_x: jax.Array,
    A_wqkv: jax.Array,
    A_wo: jax.Array,
    B_x: jax.Array,
    B_mem0: jax.Array,
    B_Wq: jax.Array,
    B_Wk: jax.Array,
    B_Wv: jax.Array,
    B_Wo: jax.Array,
    B_seg_len: int,
):
    _, S, D = A_x.shape
    _, H, Dh = B_Wq.shape
    M = B_mem0.shape[1]
    HD = H * Dh
    NP = H // 2
    PW = 2 * Dh
    n_early = S // B_seg_len * B_EARLY
    n_out = 16

    def heads_major(w):
        return w.transpose(1, 2, 0).reshape(HD, D)

    qkv_set = pltpu.VMEM((3 * D // LANES, A_HALO + A_ROWS, LANES), F32)
    out = pl.pallas_call(
        functools.partial(_kernel, seg=B_seg_len, head_dim=Dh),
        out_shape=jax.ShapeDtypeStruct((S, 2 * D), BF16),
        in_specs=[pl.BlockSpec(memory_space=pltpu.HBM)] * 9,
        out_specs=pl.BlockSpec(memory_space=pltpu.HBM),
        scratch_shapes=[
            pltpu.VMEM((S, D), BF16),
            pltpu.VMEM((3, D, D), BF16),
            pltpu.VMEM((D, D), BF16),
            pltpu.VMEM((D // LANES, D, LANES), F32),
            pltpu.VMEM((3 * D // 2, D), U32),
            pltpu.VMEM((D // 2, D), U32),
            qkv_set,
            qkv_set,
            pltpu.VMEM((A_SLOTS, A_WIN, A_GROUP, LANES), F32),
            pltpu.VMEM((S, D), BF16),
            pltpu.VMEM((S, D), BF16),
            pltpu.VMEM((M, D), BF16),
            pltpu.VMEM((HD, D), BF16),
            pltpu.VMEM((HD, D), BF16),
            pltpu.VMEM((HD, D), BF16),
            pltpu.VMEM((HD, D), BF16),
            pltpu.VMEM((NP, D // 2, PW), U32),
            pltpu.VMEM((NP, D // 2, PW), U32),
            pltpu.VMEM((NP, D // 2, PW), U32),
            pltpu.VMEM((NP, PW // 2, D), U32),
            pltpu.VMEM((n_early, D), F32),
            pltpu.VMEM((NP, n_early, PW), F32),
            pltpu.VMEM((S, 2 * D), BF16),
            pltpu.SemaphoreType.DMA((8,)),
            pltpu.SemaphoreType.DMA((4 * NP,)),
            pltpu.SemaphoreType.DMA((n_out,)),
        ],
        compiler_params=pltpu.CompilerParams(vmem_limit_bytes=120 * 1024 * 1024),
    )(
        A_x.reshape(S, D), A_wqkv, A_wo, B_x.reshape(S, D), B_mem0.reshape(M, D),
        heads_major(B_Wq), heads_major(B_Wk), heads_major(B_Wv), B_Wo.reshape(HD, D),
    )
    return out.reshape(1, S, 2 * D)
```

```python
import contextlib
import functools

import jax
import jax.numpy as jnp
from jax import lax
import jax.experimental.pallas as pl
import jax.experimental.pallas.tpu as pltpu

BF16 = jnp.bfloat16
F32 = jnp.float32
U32 = jnp.uint32

_NN = (((1,), (0,)), ((), ()))
_NT = (((1,), (1,)), ((), ()))

LANES = 128
NEG = -1000000000.0

A_HEADS = 32
A_WIN = 8
A_DIL = 2
A_HALO = 16
A_ROWS = 128
B_EARLY = 8
B_UNROLL = 4
A_SLOTS = 3
A_GROUP = 8


_SCOPES = False


def _scope(name):
    return jax.named_scope(name) if _SCOPES else contextlib.nullcontext()


def _dot(a, b, dn=_NN):
    return lax.dot_general(a, b, dn, preferred_element_type=F32)


def _pack(x):
    return pltpu.bitcast(x, U32)


def _unpack(x):
    return pltpu.bitcast(x, BF16)


B_ORDER = ("kqvpso", 5, 1, 0, 3)


def _b_order(n):
    pattern, lag_o, lag_p, lag_s, n_before = B_ORDER
    lag = dict(q=0, k=0, v=0, s=lag_s, p=lag_p, o=lag_o)
    order = []
    for t in range(n):
        for op in pattern:
            if t - lag[op] >= 0:
                order.append((op, t - lag[op]))
    rest_o = [("o", j) for j in range(n - lag_o, n)]
    for j in range(n - lag_s, n):
        order.append(rest_o.pop(0))
        order.append(("s", j))
    for j in range(n - lag_p, n - 1):
        order.append(rest_o.pop(0))
        order.append(("p", j))
    order += rest_o[:n_before] + [("p", n - 1)] + rest_o[n_before:]
    return order


def _kernel(
    xa_hbm, wqkv_hbm, woa_hbm, xb_hbm, mem_hbm, wq_hbm, wk_hbm, wv_hbm, wo_hbm,
    out_hbm,
    xa_v, wqkv_raw, woa_raw, perm_v, wqkv_p, woa_p, set_e, set_o, slot_v, oa_v,
    xb_v, mem_v, wq_raw, wk_raw, wv_raw, wo_raw, wq_p, wk_p, wv_p, wo_p,
    xq_v, early_q, early_k, out_v,
    sem_a, sem_x, sem_w, sem_o,
    *, seg, head_dim,
):
    S, D = xa_v.shape
    M = mem_v.shape[0]
    L = M + seg
    PW = 2 * head_dim
    NP = wq_p.shape[0]
    E = B_EARLY
    ppi = 2
    n_prep = NP // ppi
    n_seg = S // seg
    NT = D // LANES
    R = A_ROWS
    n_it = S // (2 * R)

    def qkv_copy(i):
        cols = pl.ds(pl.multiple_of(i * D, D), D)
        return pltpu.make_async_copy(wqkv_hbm.at[:, cols], wqkv_raw.at[i], sem_a.at[i])

    woa_copy = pltpu.make_async_copy(woa_hbm, woa_raw, sem_a.at[3])
    xb_copy = pltpu.make_async_copy(xb_hbm, xb_v, sem_a.at[4])
    mem_copy = pltpu.make_async_copy(mem_hbm, mem_v, sem_a.at[5])

    def xa_copy(i):
        rows = pl.ds(pl.multiple_of(i * 2 * R, 2 * R), 2 * R)
        return pltpu.make_async_copy(xa_hbm.at[rows], xa_v.at[rows], sem_x.at[i])

    def w_copies(j):
        rows = pl.ds(pl.multiple_of(j * ppi * PW, ppi * PW), ppi * PW)
        return [
            pltpu.make_async_copy(wq_hbm.at[rows], wq_raw.at[rows], sem_w.at[4 * j]),
            pltpu.make_async_copy(wk_hbm.at[rows], wk_raw.at[rows], sem_w.at[4 * j + 1]),
            pltpu.make_async_copy(wv_hbm.at[rows], wv_raw.at[rows], sem_w.at[4 * j + 2]),
            pltpu.make_async_copy(wo_hbm.at[rows], wo_raw.at[rows], sem_w.at[4 * j + 3]),
        ]

    def start_in_order(lo, hi, copies):
        def body(i, carry):
            for c in copies(i):
                c.start(priority=1)
            return carry
        lax.fori_loop(lo, hi, body, 0)

    for c in (qkv_copy(0), xa_copy(0)):
        c.start(priority=1)
    start_in_order(1, 3, lambda i: [qkv_copy(i)])
    start_in_order(1, n_it, lambda i: [xa_copy(i)])
    for c in (woa_copy, xb_copy, mem_copy):
        c.start(priority=1)
    start_in_order(0, n_prep, w_copies)

    dh = D // A_HEADS

    def permute_rows(w):
        w = w.astype(F32)
        for t in range(NT):
            perm_v[t] = w[:, t * LANES:(t + 1) * LANES]
        cols = [
            jnp.concatenate(
                [perm_v[t, pl.ds(d, A_HEADS, stride=dh), :] for d in range(dh)], axis=0)
            for t in range(NT)
        ]
        return _pack(jnp.concatenate(cols, axis=1).astype(BF16))

    def prepare_qkv(i):
        wqkv_p[i * D // 2:(i + 1) * D // 2, :] = permute_rows(wqkv_raw[i].T)

    a_scale = dh ** -0.5

    def a_proj(c, dst):
        x = xa_v[pl.ds(pl.multiple_of(c * R, R), R), :]
        qkv = _dot(x, _unpack(wqkv_p[...]), _NT)
        for t in range(3 * NT):
            dst[t, A_HALO:, :] = qkv[:, t * LANES:(t + 1) * LANES]

    def a_halo(src, dst):
        for t in range(NT, 3 * NT):
            dst[t, :A_HALO, :] = src[t, R:, :]

    def a_attn(c, src, first):
        G = A_GROUP

        def scores(g):
            top = A_HALO + g * G
            for t in range(NT):
                slot_v[g % A_SLOTS, t] = src[t, top:top + G, :]
            q = [slot_v[g % A_SLOTS, t] for t in range(NT)]
            out = []
            for w in range(A_WIN):
                lo = top - A_DIL * w
                s = q[0] * src[NT, lo:lo + G, :]
                for t in range(1, NT):
                    s = s + q[t] * src[NT + t, lo:lo + G, :]
                out.append(s + pltpu.roll(s, 2 * A_HEADS, 1))
            return out

        def fold(g, part):
            out = []
            for w, s in enumerate(part):
                s = (s + pltpu.roll(s, A_HEADS, 1)) * a_scale
                if first and g * G < A_DIL * w:
                    row = g * G + lax.broadcasted_iota(jnp.int32, (G, LANES), 0)
                    s = jnp.where(row >= A_DIL * w, s, NEG)
                out.append(s)
            return out

        def softmax(logits):
            mx = functools.reduce(jnp.maximum, logits)
            e = [jnp.exp(s - mx) for s in logits]
            inv = 1.0 / functools.reduce(jnp.add, e)
            return [x * inv for x in e]

        def values(g, p):
            top = A_HALO + g * G
            for w in range(A_WIN):
                slot_v[g % A_SLOTS, w] = p[w]
            p = [slot_v[g % A_SLOTS, w] for w in range(A_WIN)]
            o = []
            for t in range(NT):
                acc = p[0] * src[2 * NT + t, top:top + G, :]
                for w in range(1, A_WIN):
                    lo = top - A_DIL * w
                    acc = acc + p[w] * src[2 * NT + t, lo:lo + G, :]
                o.append(acc)
            return jnp.concatenate(o, axis=1)

        n = R // G
        per = max(1, 16 // G)
        st = {}
        for u in range(n):
            st[u] = softmax(fold(u, scores(u)))
            g = u
            if 0 <= g < n:
                st[g] = values(g, st[g])
                if g % per == per - 1:
                    g0 = g - per + 1
                    oa_v[pl.ds(pl.multiple_of(c * R + g0 * G, per * G), per * G), :] = (
                        jnp.concatenate([st[i] for i in range(g0, g + 1)], axis=0).astype(BF16))

    with _scope("a_it0"):
        qkv_copy(0).wait()
        prepare_qkv(0)
        xa_copy(0).wait()
        for i in range(3):
            if i < 2:
                qkv_copy(i + 1).wait()
            part = _dot(xa_v[:2 * R, :],
                        _unpack(wqkv_p[i * D // 2:(i + 1) * D // 2, :]), _NT)
            for t in range(NT):
                set_e[i * NT + t, A_HALO:, :] = part[:R, t * LANES:(t + 1) * LANES]
                set_o[i * NT + t, A_HALO:, :] = part[R:, t * LANES:(t + 1) * LANES]
            if i < 2:
                prepare_qkv(i + 1)
        for t in range(NT, 3 * NT):
            set_e[t, :A_HALO, :] = jnp.broadcast_to(
                set_e[t, A_HALO:A_HALO + 1, :], (A_HALO, LANES))
        a_halo(set_e, set_o)
        a_attn(0, set_e, True)


    def a_loop(i, carry):
        with _scope("a_it"):
            xa_copy(i).wait()
            a_halo(set_o, set_e)
            a_attn(2 * i - 1, set_o, False)
            a_proj(2 * i, set_e)
            a_halo(set_e, set_o)
            a_attn(2 * i, set_e, False)
            a_proj(2 * i + 1, set_o)
        return carry

    lax.fori_loop(1, n_it, a_loop, 0)
    with _scope("a_end"):
        xb_copy.wait()
        mem_copy.wait()
        woa_copy.wait()
        for c in w_copies(0):
            c.wait()
        woa_p[...] = permute_rows(woa_raw[...])
        a_attn(2 * n_it - 1, set_o, False)
        for s in range(n_seg):
            xq_v[s * E:(s + 1) * E, :] = xb_v[(s + 1) * seg - E:(s + 1) * seg, :].astype(F32)
        for j in range(early_k.shape[0]):
            early_k[j] = _dot(xq_v[...], wk_raw[j * PW:(j + 1) * PW, :], _NT)


    def b_prep(i, carry):
        with _scope("b_prep"):
            for jj in range(ppi):
                j = i * ppi + jj
                rows = pl.ds(pl.multiple_of(j * PW, PW), PW)
                early_q[j] = _dot(xq_v[...], wq_raw[rows, :], _NT)
                wq_p[j] = _pack(wq_raw[rows, :].T)
                wk_p[j] = _pack(wk_raw[rows, :].T)
                wv_p[j] = _pack(wv_raw[rows, :].T)
                wo_p[j] = _pack(wo_raw[rows, :])

            @pl.when(i + 1 < n_prep)
            def _():
                for c in w_copies(i + 1):
                    c.wait()
        return carry

    lax.fori_loop(0, n_prep, b_prep, 0)

    b_scale = head_dim ** -0.5

    order = _b_order(NP)

    def b_step(s, mem):
        r0 = pl.multiple_of(s * seg, seg)
        h = jnp.concatenate([mem, xb_v[pl.ds(r0, seg), :].astype(F32)], axis=0)
        lane = lax.broadcasted_iota(jnp.int32, (L, LANES), 1)
        row = lax.broadcasted_iota(jnp.int32, (L, LANES), 0)
        is_a = lane < L
        is_b = (lane >= L) & (lane < 2 * L)
        visible = (row < M) | (row >= jnp.where(is_a, lane, lane - L))
        feat_a = lax.broadcasted_iota(jnp.int32, (L, PW), 1) < head_dim

        def block_diag(t):
            return jnp.concatenate(
                [jnp.where(feat_a, t, 0.0), jnp.where(feat_a, 0.0, t),
                 jnp.zeros((LANES - 2 * L, PW), F32)], axis=0).astype(BF16)

        q, k, v, p, o = {}, {}, {}, {}, {}
        acc = None
        for op, j in order:
            if op == "q":
                q[j] = jnp.concatenate(
                    [_dot(h[:L - E], _unpack(wq_p[j])),
                     early_q[j, pl.ds(pl.multiple_of(s * E, E), E), :]], axis=0)
            elif op == "k":
                if j < early_k.shape[0]:
                    k[j] = jnp.concatenate(
                        [_dot(h[:L - E], _unpack(wk_p[j])),
                         early_k[j, pl.ds(pl.multiple_of(s * E, E), E), :]], axis=0)
                else:
                    k[j] = _dot(h, _unpack(wk_p[j]))
            elif op == "v":
                v[j] = _dot(h, _unpack(wv_p[j]))
            elif op == "s":
                sc = _dot(q[j], block_diag(k[j]), _NT) * b_scale
                sc = jnp.where(visible, sc, NEG)
                m_a = jnp.max(jnp.where(is_a, sc, -jnp.inf), axis=1, keepdims=True)
                m_b = jnp.max(jnp.where(is_b, sc, -jnp.inf), axis=1, keepdims=True)
                e = jnp.exp(sc - jnp.where(is_a, m_a, m_b))
                e_a = jnp.where(is_a, e, 0.0)
                e_b = jnp.where(is_b, e, 0.0)
                l_a = jnp.sum(e_a, axis=1, keepdims=True)
                l_b = jnp.sum(e_b, axis=1, keepdims=True)
                p[j] = (e_a + e_b) / jnp.where(is_a, l_a, l_b)
            elif op == "p":
                o[j] = _dot(p[j], block_diag(v[j]))
            else:
                d = _dot(o[j], _unpack(wo_p[j]))
                acc = d if acc is None else acc + d
        out_v[pl.ds(r0, seg), D:] = acc[M:].astype(BF16)
        out_v[pl.ds(r0, seg), :D] = _dot(
            oa_v[pl.ds(r0, seg), :], _unpack(woa_p[...])).astype(BF16)
        return acc[:M]

    n_out = sem_o.shape[0]
    spo = n_seg // n_out

    def outb_copy(i):
        rows = pl.ds(pl.multiple_of(i * spo * seg, spo * seg), spo * seg)
        return pltpu.make_async_copy(
            out_v.at[rows], out_hbm.at[rows], sem_o.at[i])

    def b_outer(i, mem):
        with _scope("b_outer"):
            mem = lax.fori_loop(0, spo, lambda u, m: b_step(i * spo + u, m), mem, unroll=B_UNROLL)
        outb_copy(i).start()
        return mem

    lax.fori_loop(0, n_out, b_outer, mem_v[...].astype(F32))

    for i in range(n_out):
        outb_copy(i).wait()


@functools.partial(jax.jit, static_argnames=("B_seg_len",))
def pallas_concat_heads__sliding_local_dilated__memory_aug_recurrent_mem_tr__prompt_kernel(
    A_x: jax.Array,
    A_wqkv: jax.Array,
    A_wo: jax.Array,
    B_x: jax.Array,
    B_mem0: jax.Array,
    B_Wq: jax.Array,
    B_Wk: jax.Array,
    B_Wv: jax.Array,
    B_Wo: jax.Array,
    B_seg_len: int,
):
    _, S, D = A_x.shape
    _, H, Dh = B_Wq.shape
    M = B_mem0.shape[1]
    HD = H * Dh
    NP = H // 2
    PW = 2 * Dh
    n_early = S // B_seg_len * B_EARLY
    n_out = 16

    def heads_major(w):
        return w.transpose(1, 2, 0).reshape(HD, D)

    qkv_set = pltpu.VMEM((3 * D // LANES, A_HALO + A_ROWS, LANES), F32)
    out = pl.pallas_call(
        functools.partial(_kernel, seg=B_seg_len, head_dim=Dh),
        out_shape=jax.ShapeDtypeStruct((S, 2 * D), BF16),
        in_specs=[pl.BlockSpec(memory_space=pltpu.HBM)] * 9,
        out_specs=pl.BlockSpec(memory_space=pltpu.HBM),
        scratch_shapes=[
            pltpu.VMEM((S, D), BF16),
            pltpu.VMEM((3, D, D), BF16),
            pltpu.VMEM((D, D), BF16),
            pltpu.VMEM((D // LANES, D, LANES), F32),
            pltpu.VMEM((3 * D // 2, D), U32),
            pltpu.VMEM((D // 2, D), U32),
            qkv_set,
            qkv_set,
            pltpu.VMEM((A_SLOTS, A_WIN, A_GROUP, LANES), F32),
            pltpu.VMEM((S, D), BF16),
            pltpu.VMEM((S, D), BF16),
            pltpu.VMEM((M, D), BF16),
            pltpu.VMEM((HD, D), BF16),
            pltpu.VMEM((HD, D), BF16),
            pltpu.VMEM((HD, D), BF16),
            pltpu.VMEM((HD, D), BF16),
            pltpu.VMEM((NP, D // 2, PW), U32),
            pltpu.VMEM((NP, D // 2, PW), U32),
            pltpu.VMEM((NP, D // 2, PW), U32),
            pltpu.VMEM((NP, PW // 2, D), U32),
            pltpu.VMEM((n_early, D), F32),
            pltpu.VMEM((NP, n_early, PW), F32),
            pltpu.VMEM((1, n_early, PW), F32),
            pltpu.VMEM((S, 2 * D), BF16),
            pltpu.SemaphoreType.DMA((6,)),
            pltpu.SemaphoreType.DMA((S // (2 * A_ROWS),)),
            pltpu.SemaphoreType.DMA((4 * NP // 2,)),
            pltpu.SemaphoreType.DMA((n_out,)),
        ],
        compiler_params=pltpu.CompilerParams(vmem_limit_bytes=120 * 1024 * 1024),
    )(
        A_x.reshape(S, D), A_wqkv, A_wo, B_x.reshape(S, D), B_mem0.reshape(M, D),
        heads_major(B_Wq), heads_major(B_Wk), heads_major(B_Wv), B_Wo.reshape(HD, D),
    )
    return out.reshape(1, S, 2 * D)
```

```python
import functools

import jax
import jax.numpy as jnp
from jax import lax
import jax.experimental.pallas as pl
import jax.experimental.pallas.tpu as pltpu

BF16 = jnp.bfloat16
F32 = jnp.float32
U32 = jnp.uint32

_NN = (((1,), (0,)), ((), ()))
_NT = (((1,), (1,)), ((), ()))

LANES = 128
MASKED = -1000000000.0

A_HEADS = 32
A_WIN = 8
A_DIL = 2

A_HALO = 16
A_ROWS = 128
A_GROUP = 8
A_SLOTS = 3
PERM_PAD = 24
B_EARLY = 8
B_EARLY_K = 1
B_PAIRS = 2
B_UNROLL = 4


def _dot(a, b, dn=_NN):
    return lax.dot_general(a, b, dn, preferred_element_type=F32)


def _pack(x):
    return pltpu.bitcast(x, U32)


def _unpack(x):
    return pltpu.bitcast(x, BF16)


def _b_order(n):
    lag = dict(k=0, s=1, q=0, p=2, v=0, o=6)
    order = [(op, t - lag[op]) for t in range(n) for op in "ksqpvo" if t >= lag[op]]
    return order + [
        ("o", n - 6), ("s", n - 1), ("o", n - 5), ("p", n - 2), ("o", n - 4),
        ("o", n - 3), ("p", n - 1), ("o", n - 2), ("o", n - 1),
    ]


def _kernel(
    xa_hbm, wqkv_hbm, woa_hbm, xb_hbm, mem_hbm, wq_hbm, wk_hbm, wv_hbm, wo_hbm,
    out_hbm,
    xa_v, wqkv_raw, woa_raw, perm_v, wqkv_p, woa_p, set_e, set_o, slot_v, oa_v,
    xb_v, mem_v, wq_raw, wk_raw, wv_raw, wo_raw, wq_p, wk_p, wv_p, wo_p,
    xe_v, early_q, early_k, out_v,
    sem_a, sem_x, sem_w, sem_o,
    *, seg, head_dim,
):
    S, D = xa_v.shape
    M = mem_v.shape[0]
    L = M + seg
    PW = 2 * head_dim
    NP = wq_p.shape[0]
    NT = D // LANES
    R = A_ROWS
    E = B_EARLY
    n_a = S // (2 * R)
    n_seg = S // seg
    n_prep = NP // B_PAIRS

    def qkv_copy(i):
        cols = pl.ds(pl.multiple_of(i * D, D), D)
        return pltpu.make_async_copy(wqkv_hbm.at[:, cols], wqkv_raw.at[i], sem_a.at[i])

    woa_copy = pltpu.make_async_copy(woa_hbm, woa_raw, sem_a.at[3])
    xb_copy = pltpu.make_async_copy(xb_hbm, xb_v, sem_a.at[4])
    mem_copy = pltpu.make_async_copy(mem_hbm, mem_v, sem_a.at[5])

    def xa_copy(i):
        rows = pl.ds(pl.multiple_of(i * 2 * R, 2 * R), 2 * R)
        return pltpu.make_async_copy(xa_hbm.at[rows], xa_v.at[rows], sem_x.at[i])

    def w_copies(i):
        rows = pl.ds(pl.multiple_of(i * B_PAIRS * PW, B_PAIRS * PW), B_PAIRS * PW)
        return [
            pltpu.make_async_copy(src.at[rows], dst.at[rows], sem_w.at[i])
            for src, dst in ((wq_hbm, wq_raw), (wk_hbm, wk_raw),
                             (wv_hbm, wv_raw), (wo_hbm, wo_raw))
        ]

    def wait_weights(i):
        for c in w_copies(i):
            c.wait()

    def start_in_order(lo, hi, copies):
        def body(i, carry):
            for c in copies(i):
                c.start(priority=1)
            return carry
        lax.fori_loop(lo, hi, body, 0)

    for c in (qkv_copy(0), xa_copy(0)):
        c.start(priority=1)
    start_in_order(1, 3, lambda i: [qkv_copy(i)])
    start_in_order(1, n_a, lambda i: [xa_copy(i)])
    for c in (woa_copy, xb_copy, mem_copy):
        c.start(priority=1)
    start_in_order(0, n_prep, w_copies)

    dh = D // A_HEADS
    a_scale = dh ** -0.5

    def permute_rows(w):
        w = w.astype(F32)
        for t in range(NT):
            perm_v[t, :D, :] = w[:, t * LANES:(t + 1) * LANES]
        cols = [
            jnp.concatenate(
                [perm_v[t, pl.ds(d, A_HEADS, stride=dh), :] for d in range(dh)], axis=0)
            for t in range(NT)
        ]
        return _pack(jnp.concatenate(cols, axis=1).astype(BF16))

    def prepare_qkv(i):
        wqkv_p[i * D // 2:(i + 1) * D // 2, :] = permute_rows(wqkv_raw[i].T)

    def a_project(c, dst):
        x = xa_v[pl.ds(pl.multiple_of(c * R, R), R), :]
        qkv = _dot(x, _unpack(wqkv_p[...]), _NT)
        for t in range(3 * NT):
            dst[t, A_HALO:, :] = qkv[:, t * LANES:(t + 1) * LANES]

    def a_halo(src, dst):
        for t in range(NT, 3 * NT):
            dst[t, :A_HALO, :] = src[t, R:, :]

    def a_attend_group(src, g, first):
        G = A_GROUP
        top = A_HALO + g * G
        slot = g % A_SLOTS

        def window(t, w):
            return src[t, top - A_DIL * w:top - A_DIL * w + G, :]

        for t in range(NT):
            slot_v[slot, t] = window(t, 0)
        q = [slot_v[slot, t] for t in range(NT)]
        logits = []
        for w in range(A_WIN):
            s = functools.reduce(jnp.add, [q[t] * window(NT + t, w) for t in range(NT)])
            logits.append(s + pltpu.roll(s, 2 * A_HEADS, 1))
        for w, s in enumerate(logits):
            s = (s + pltpu.roll(s, A_HEADS, 1)) * a_scale
            if first and g * G < A_DIL * w:
                row = g * G + lax.broadcasted_iota(jnp.int32, (G, LANES), 0)
                s = jnp.where(row >= A_DIL * w, s, MASKED)
            logits[w] = s
        mx = functools.reduce(jnp.maximum, logits)
        e = [jnp.exp(s - mx) for s in logits]
        inv = 1.0 / functools.reduce(jnp.add, e)
        for w in range(A_WIN):
            slot_v[slot, w] = e[w] * inv
        p = [slot_v[slot, w] for w in range(A_WIN)]
        return jnp.concatenate(
            [functools.reduce(
                jnp.add, [p[w] * window(2 * NT + t, w) for w in range(A_WIN)])
             for t in range(NT)], axis=1)

    def a_attend(c, src, first=False):
        for g in range(0, R // A_GROUP, 2):
            o = jnp.concatenate(
                [a_attend_group(src, g, first), a_attend_group(src, g + 1, first)],
                axis=0)
            row0 = pl.multiple_of(c * R + g * A_GROUP, 2 * A_GROUP)
            oa_v[pl.ds(row0, 2 * A_GROUP), :] = o.astype(BF16)

    perm_v[:, D:, :] = jnp.zeros((NT, PERM_PAD, LANES), F32)
    qkv_copy(0).wait()
    prepare_qkv(0)
    xa_copy(0).wait()
    for i in range(3):
        if i < 2:
            qkv_copy(i + 1).wait()
        part = _dot(xa_v[:2 * R, :],
                    _unpack(wqkv_p[i * D // 2:(i + 1) * D // 2, :]), _NT)
        for t in range(NT):
            set_e[i * NT + t, A_HALO:, :] = part[:R, t * LANES:(t + 1) * LANES]
            set_o[i * NT + t, A_HALO:, :] = part[R:, t * LANES:(t + 1) * LANES]
        if i < 2:
            prepare_qkv(i + 1)
    for t in range(NT, 3 * NT):
        set_e[t, :A_HALO, :] = jnp.broadcast_to(
            set_e[t, A_HALO:A_HALO + 1, :], (A_HALO, LANES))
    a_halo(set_e, set_o)
    a_attend(0, set_e, first=True)

    def a_loop(i, carry):
        xa_copy(i).wait()
        a_halo(set_o, set_e)
        a_attend(2 * i - 1, set_o)
        a_project(2 * i, set_e)
        a_halo(set_e, set_o)
        a_attend(2 * i, set_e)
        a_project(2 * i + 1, set_o)
        return carry

    lax.fori_loop(1, n_a, a_loop, 0)

    xb_copy.wait()
    mem_copy.wait()
    woa_copy.wait()
    wait_weights(0)
    woa_p[...] = permute_rows(woa_raw[...])
    a_attend(2 * n_a - 1, set_o)

    for s in range(n_seg):
        xe_v[s * E:(s + 1) * E, :] = xb_v[(s + 1) * seg - E:(s + 1) * seg, :].astype(F32)
    for j in range(B_EARLY_K):
        early_k[j] = _dot(xe_v[...], wk_raw[j * PW:(j + 1) * PW, :], _NT)

    def b_prepare(i, carry):
        for jj in range(B_PAIRS):
            j = i * B_PAIRS + jj
            rows = pl.ds(pl.multiple_of(j * PW, PW), PW)
            early_q[j] = _dot(xe_v[...], wq_raw[rows, :], _NT)
            wq_p[j] = _pack(wq_raw[rows, :].T)
            wk_p[j] = _pack(wk_raw[rows, :].T)
            wv_p[j] = _pack(wv_raw[rows, :].T)
            wo_p[j] = _pack(wo_raw[rows, :])

        @pl.when(i + 1 < n_prep)
        def _():
            wait_weights(i + 1)

        return carry

    lax.fori_loop(0, n_prep, b_prepare, 0)

    b_scale = head_dim ** -0.5
    order = _b_order(NP)

    def b_segment(s, mem):
        rows = pl.ds(pl.multiple_of(s * seg, seg), seg)
        early_rows = pl.ds(pl.multiple_of(s * E, E), E)
        h = jnp.concatenate([mem, xb_v[rows, :].astype(F32)], axis=0)

        lane = lax.broadcasted_iota(jnp.int32, (L, LANES), 1)
        row = lax.broadcasted_iota(jnp.int32, (L, LANES), 0)
        is_a = lane < L
        is_b = (lane >= L) & (lane < 2 * L)
        visible = (row < M) | (row >= jnp.where(is_a, lane, lane - L))
        feat_a = lax.broadcasted_iota(jnp.int32, (L, PW), 1) < head_dim

        def block_diag(t):
            return jnp.concatenate(
                [jnp.where(feat_a, t, 0.0), jnp.where(feat_a, 0.0, t),
                 jnp.zeros((LANES - 2 * L, PW), F32)], axis=0).astype(BF16)

        def project(w_p, j, early=None):
            if early is None:
                return _dot(h, _unpack(w_p[j]))
            return jnp.concatenate(
                [_dot(h[:L - E], _unpack(w_p[j])), early[j, early_rows, :]], axis=0)

        def probabilities(q, k):
            sc = jnp.where(visible, _dot(q, block_diag(k), _NT) * b_scale, MASKED)
            m_a = jnp.max(jnp.where(is_a, sc, -jnp.inf), axis=1, keepdims=True)
            m_b = jnp.max(jnp.where(is_b, sc, -jnp.inf), axis=1, keepdims=True)
            e = jnp.exp(sc - jnp.where(is_a, m_a, m_b))
            e_a = jnp.where(is_a, e, 0.0)
            e_b = jnp.where(is_b, e, 0.0)
            l_a = jnp.sum(e_a, axis=1, keepdims=True)
            l_b = jnp.sum(e_b, axis=1, keepdims=True)
            return (e_a + e_b) / jnp.where(is_a, l_a, l_b)

        q, k, v, p, o = {}, {}, {}, {}, {}
        acc = None
        for op, j in order:
            if op == "q":
                q[j] = project(wq_p, j, early_q)
            elif op == "k":
                k[j] = project(wk_p, j, early_k if j < B_EARLY_K else None)
            elif op == "v":
                v[j] = project(wv_p, j)
            elif op == "s":
                p[j] = probabilities(q[j], k[j])
            elif op == "p":
                o[j] = _dot(p[j], block_diag(v[j]))
            else:
                d = _dot(o[j], _unpack(wo_p[j]))
                acc = d if acc is None else acc + d
        out_v[rows, D:] = acc[M:].astype(BF16)
        out_v[rows, :D] = _dot(oa_v[rows, :], _unpack(woa_p[...])).astype(BF16)
        pltpu.make_async_copy(out_v.at[rows], out_hbm.at[rows], sem_o.at[0]).start()
        return acc[:M]

    def b_loop(i, mem):
        for u in range(B_UNROLL):
            mem = b_segment(i * B_UNROLL + u, mem)
        return mem

    lax.fori_loop(0, n_seg // B_UNROLL, b_loop, mem_v[...].astype(F32))

    pltpu.make_async_copy(out_v, out_hbm, sem_o.at[0]).wait()


@functools.partial(jax.jit, static_argnames=("B_seg_len",))
def pallas_concat_heads__sliding_local_dilated__memory_aug_recurrent_mem_tr__prompt_kernel(
    A_x: jax.Array,
    A_wqkv: jax.Array,
    A_wo: jax.Array,
    B_x: jax.Array,
    B_mem0: jax.Array,
    B_Wq: jax.Array,
    B_Wk: jax.Array,
    B_Wv: jax.Array,
    B_Wo: jax.Array,
    B_seg_len: int,
):
    batch, S, D = A_x.shape
    _, H, Dh = B_Wq.shape
    M = B_mem0.shape[1]
    HD = H * Dh
    NP = H // 2
    PW = 2 * Dh
    NT = D // LANES
    n_early = S // B_seg_len * B_EARLY
    assert batch == 1 and B_x.shape == A_x.shape
    assert D % LANES == 0 and PW % LANES == 0 and NT <= A_WIN
    assert S % (2 * A_ROWS) == 0 and S % (B_UNROLL * B_seg_len) == 0
    assert M % 8 == 0 and B_seg_len % 16 == 0 and 2 * (M + B_seg_len) < LANES
    assert NP % B_PAIRS == 0 and NP > 6

    def heads_major(w):
        return w.transpose(1, 2, 0).reshape(HD, D)

    qkv_set = pltpu.VMEM((3 * NT, A_HALO + A_ROWS, LANES), F32)
    out = pl.pallas_call(
        functools.partial(_kernel, seg=B_seg_len, head_dim=Dh),
        out_shape=jax.ShapeDtypeStruct((S, 2 * D), BF16),
        in_specs=[pl.BlockSpec(memory_space=pltpu.HBM)] * 9,
        out_specs=pl.BlockSpec(memory_space=pltpu.HBM),
        scratch_shapes=[
            pltpu.VMEM((S, D), BF16),
            pltpu.VMEM((3, D, D), BF16),
            pltpu.VMEM((D, D), BF16),
            pltpu.VMEM((NT, D + PERM_PAD, LANES), F32),
            pltpu.VMEM((3 * D // 2, D), U32),
            pltpu.VMEM((D // 2, D), U32),
            qkv_set,
            qkv_set,
            pltpu.VMEM((A_SLOTS, A_WIN, A_GROUP, LANES), F32),
            pltpu.VMEM((S, D), BF16),
            pltpu.VMEM((S, D), BF16),
            pltpu.VMEM((M, D), BF16),
            pltpu.VMEM((HD, D), BF16),
            pltpu.VMEM((HD, D), BF16),
            pltpu.VMEM((HD, D), BF16),
            pltpu.VMEM((HD, D), BF16),
            pltpu.VMEM((NP, D // 2, PW), U32),
            pltpu.VMEM((NP, D // 2, PW), U32),
            pltpu.VMEM((NP, D // 2, PW), U32),
            pltpu.VMEM((NP, PW // 2, D), U32),
            pltpu.VMEM((n_early, D), F32),
            pltpu.VMEM((NP, n_early, PW), F32),
            pltpu.VMEM((B_EARLY_K, n_early, PW), F32),
            pltpu.VMEM((S, 2 * D), BF16),
            pltpu.SemaphoreType.DMA((6,)),
            pltpu.SemaphoreType.DMA((S // (2 * A_ROWS),)),
            pltpu.SemaphoreType.DMA((NP // B_PAIRS,)),
            pltpu.SemaphoreType.DMA((1,)),
        ],
        compiler_params=pltpu.CompilerParams(vmem_limit_bytes=120 * 1024 * 1024),
    )(
        A_x.reshape(S, D), A_wqkv, A_wo, B_x.reshape(S, D), B_mem0.reshape(M, D),
        heads_major(B_Wq), heads_major(B_Wk), heads_major(B_Wv), B_Wo.reshape(HD, D),
    )
    return out.reshape(1, S, 2 * D)
```

```python
import functools

import jax
import jax.numpy as jnp
from jax import lax
import jax.experimental.pallas as pl
import jax.experimental.pallas.tpu as pltpu

BF16 = jnp.bfloat16
F32 = jnp.float32
U32 = jnp.uint32

_NN = (((1,), (0,)), ((), ()))
_NT = (((1,), (1,)), ((), ()))

LANES = 128
MASKED = -1000000000.0

A_HEADS = 32
A_WIN = 8
A_DIL = 2

A_HALO = 16
A_ROWS = 128
A_GROUP = 8
A_SLOTS = 3
PERM_PAD = 32
B_EARLY = 8
B_EARLY_K = 2
B_PAIRS = 2
B_UNROLL = 4


def _dot(a, b, dn=_NN):
    return lax.dot_general(a, b, dn, preferred_element_type=F32)


def _pack(x):
    return pltpu.bitcast(x, U32)


def _unpack(x):
    return pltpu.bitcast(x, BF16)


def _b_order(n):
    lag = dict(k=0, s=1, q=0, p=2, v=0, o=6)
    order = [(op, t - lag[op]) for t in range(n) for op in "ksqpvo" if t >= lag[op]]
    return order + [
        ("o", n - 6), ("s", n - 1), ("o", n - 5), ("p", n - 2), ("o", n - 4),
        ("o", n - 3), ("p", n - 1), ("o", n - 2), ("o", n - 1),
    ]


def _kernel(
    xa_hbm, wqkv_hbm, woa_hbm, xb_hbm, mem_hbm, wq_hbm, wk_hbm, wv_hbm, wo_hbm,
    out_hbm,
    xa_v, wqkv_raw, woa_raw, perm_v, wqkv_p, woa_p, set_e, set_o, slot_v, oa_v,
    xb_v, mem_v, wq_raw, wk_raw, wv_raw, wo_raw, wq_p, wk_p, wv_p, wo_p,
    xe_v, early_q, early_k, out_v,
    sem_a, sem_x, sem_w, sem_o,
    *, seg, head_dim,
):
    S, D = xa_v.shape
    M = mem_v.shape[0]
    L = M + seg
    PW = 2 * head_dim
    NP = wq_p.shape[0]
    NT = D // LANES
    R = A_ROWS
    E = B_EARLY
    n_a = S // (2 * R)
    n_seg = S // seg
    n_prep = NP // B_PAIRS

    def qkv_copy(i):
        cols = pl.ds(pl.multiple_of(i * D, D), D)
        return pltpu.make_async_copy(wqkv_hbm.at[:, cols], wqkv_raw.at[i], sem_a.at[i])

    woa_copy = pltpu.make_async_copy(woa_hbm, woa_raw, sem_a.at[3])
    xb_copy = pltpu.make_async_copy(xb_hbm, xb_v, sem_a.at[4])
    mem_copy = pltpu.make_async_copy(mem_hbm, mem_v, sem_a.at[5])

    def xa_copy(i):
        rows = pl.ds(pl.multiple_of(i * 2 * R, 2 * R), 2 * R)
        return pltpu.make_async_copy(xa_hbm.at[rows], xa_v.at[rows], sem_x.at[i])

    def w_copies(i):
        rows = pl.ds(pl.multiple_of(i * B_PAIRS * PW, B_PAIRS * PW), B_PAIRS * PW)
        return [
            pltpu.make_async_copy(src.at[rows], dst.at[rows], sem_w.at[i])
            for src, dst in ((wq_hbm, wq_raw), (wk_hbm, wk_raw),
                             (wv_hbm, wv_raw), (wo_hbm, wo_raw))
        ]

    def wait_weights(i):
        for c in w_copies(i):
            c.wait()

    def start_in_order(lo, hi, copies):
        def body(i, carry):
            for c in copies(i):
                c.start(priority=1)
            return carry
        lax.fori_loop(lo, hi, body, 0)

    for c in (qkv_copy(0), xa_copy(0)):
        c.start(priority=1)
    start_in_order(1, 3, lambda i: [qkv_copy(i)])
    start_in_order(1, n_a, lambda i: [xa_copy(i)])
    for c in (woa_copy, xb_copy, mem_copy):
        c.start(priority=1)
    start_in_order(0, n_prep, w_copies)

    dh = D // A_HEADS
    a_scale = dh ** -0.5

    def permute_rows(w):
        w = w.astype(F32)
        for t in range(NT):
            perm_v[t, :D, :] = w[:, t * LANES:(t + 1) * LANES]
        cols = [
            jnp.concatenate(
                [perm_v[t, pl.ds(d, A_HEADS, stride=dh), :] for d in range(dh)], axis=0)
            for t in range(NT)
        ]
        return _pack(jnp.concatenate(cols, axis=1).astype(BF16))

    def prepare_qkv(i):
        wqkv_p[i * D // 2:(i + 1) * D // 2, :] = permute_rows(wqkv_raw[i].T)

    def a_project(c, dst):
        x = xa_v[pl.ds(pl.multiple_of(c * R, R), R), :]
        qkv = _dot(x, _unpack(wqkv_p[...]), _NT)
        for t in range(3 * NT):
            dst[t, A_HALO:, :] = qkv[:, t * LANES:(t + 1) * LANES]

    def a_halo(src, dst):
        for t in range(NT, 3 * NT):
            dst[t, :A_HALO, :] = src[t, R:, :]

    def a_attend_group(src, g, first):
        G = A_GROUP
        top = A_HALO + g * G
        slot = g % A_SLOTS

        def window(t, w):
            return src[t, top - A_DIL * w:top - A_DIL * w + G, :]

        for t in range(NT):
            slot_v[slot, t] = window(t, 0)
        q = [slot_v[slot, t] for t in range(NT)]
        logits = []
        for w in range(A_WIN):
            s = functools.reduce(jnp.add, [q[t] * window(NT + t, w) for t in range(NT)])
            logits.append(s + pltpu.roll(s, 2 * A_HEADS, 1))
        for w, s in enumerate(logits):
            s = (s + pltpu.roll(s, A_HEADS, 1)) * a_scale
            if first and g * G < A_DIL * w:
                row = g * G + lax.broadcasted_iota(jnp.int32, (G, LANES), 0)
                s = jnp.where(row >= A_DIL * w, s, MASKED)
            logits[w] = s
        mx = functools.reduce(jnp.maximum, logits)
        e = [jnp.exp(s - mx) for s in logits]
        inv = 1.0 / functools.reduce(jnp.add, e)
        for w in range(A_WIN):
            slot_v[slot, w] = e[w] * inv
        p = [slot_v[slot, w] for w in range(A_WIN)]
        return jnp.concatenate(
            [functools.reduce(
                jnp.add, [p[w] * window(2 * NT + t, w) for w in range(A_WIN)])
             for t in range(NT)], axis=1)

    def a_attend(c, src, first=False):
        for g in range(0, R // A_GROUP, 2):
            o = jnp.concatenate(
                [a_attend_group(src, g, first), a_attend_group(src, g + 1, first)],
                axis=0)
            row0 = pl.multiple_of(c * R + g * A_GROUP, 2 * A_GROUP)
            oa_v[pl.ds(row0, 2 * A_GROUP), :] = o.astype(BF16)

    perm_v[:, D:, :] = jnp.zeros((NT, PERM_PAD, LANES), F32)
    qkv_copy(0).wait()
    prepare_qkv(0)
    xa_copy(0).wait()
    for i in range(3):
        if i < 2:
            qkv_copy(i + 1).wait()
        part = _dot(xa_v[:2 * R, :],
                    _unpack(wqkv_p[i * D // 2:(i + 1) * D // 2, :]), _NT)
        for t in range(NT):
            set_e[i * NT + t, A_HALO:, :] = part[:R, t * LANES:(t + 1) * LANES]
            set_o[i * NT + t, A_HALO:, :] = part[R:, t * LANES:(t + 1) * LANES]
        if i < 2:
            prepare_qkv(i + 1)
    for t in range(NT, 3 * NT):
        set_e[t, :A_HALO, :] = jnp.broadcast_to(
            set_e[t, A_HALO:A_HALO + 1, :], (A_HALO, LANES))
    a_halo(set_e, set_o)
    a_attend(0, set_e, first=True)

    def a_loop(i, carry):
        xa_copy(i).wait()
        a_halo(set_o, set_e)
        a_attend(2 * i - 1, set_o)
        a_project(2 * i, set_e)
        a_halo(set_e, set_o)
        a_attend(2 * i, set_e)
        a_project(2 * i + 1, set_o)
        return carry

    lax.fori_loop(1, n_a, a_loop, 0)

    xb_copy.wait()
    mem_copy.wait()
    woa_copy.wait()
    wait_weights(0)
    woa_p[...] = permute_rows(woa_raw[...])
    a_attend(2 * n_a - 1, set_o)

    for s in range(0, n_seg, 2):
        tails = [xb_v[(i + 1) * seg - E:(i + 1) * seg, :].astype(F32) for i in (s, s + 1)]
        xe_v[s * E // 2:(s + 2) * E // 2, :] = _pack(
            jnp.concatenate(tails, axis=0).astype(BF16))
    for j in range(B_EARLY_K):
        early_k[j] = _dot(_unpack(xe_v[...]), wk_raw[j * PW:(j + 1) * PW, :], _NT)

    def b_prepare(i, carry):
        for jj in range(B_PAIRS):
            j = i * B_PAIRS + jj
            rows = pl.ds(pl.multiple_of(j * PW, PW), PW)
            early_q[j] = _dot(_unpack(xe_v[...]), wq_raw[rows, :], _NT)
            wq_p[j] = _pack(wq_raw[rows, :].T)
            wk_p[j] = _pack(wk_raw[rows, :].T)
            wv_p[j] = _pack(wv_raw[rows, :].T)
            wo_p[j] = _pack(wo_raw[rows, :])

        @pl.when(i + 1 < n_prep)
        def _():
            wait_weights(i + 1)

        return carry

    lax.fori_loop(0, n_prep, b_prepare, 0)

    b_scale = head_dim ** -0.5
    order = _b_order(NP)

    def b_segment(s, mem):
        rows = pl.ds(pl.multiple_of(s * seg, seg), seg)
        early_rows = pl.ds(pl.multiple_of(s * E, E), E)
        h = jnp.concatenate([mem, xb_v[rows, :].astype(F32)], axis=0)

        lane = lax.broadcasted_iota(jnp.int32, (L, LANES), 1)
        row = lax.broadcasted_iota(jnp.int32, (L, LANES), 0)
        is_a = lane < L
        is_b = (lane >= L) & (lane < 2 * L)
        visible = (row < M) | (row >= jnp.where(is_a, lane, lane - L))
        feat_a = lax.broadcasted_iota(jnp.int32, (L, PW), 1) < head_dim

        def block_diag(t):
            return jnp.concatenate(
                [jnp.where(feat_a, t, 0.0), jnp.where(feat_a, 0.0, t),
                 jnp.zeros((LANES - 2 * L, PW), F32)], axis=0).astype(BF16)

        def project(w_p, j, early=None):
            if early is None:
                return _dot(h, _unpack(w_p[j]))
            return jnp.concatenate(
                [_dot(h[:L - E], _unpack(w_p[j])), early[j, early_rows, :]], axis=0)

        def probabilities(q, k):
            sc = jnp.where(visible, _dot(q, block_diag(k), _NT) * b_scale, MASKED)
            m_a = jnp.max(jnp.where(is_a, sc, -jnp.inf), axis=1, keepdims=True)
            m_b = jnp.max(jnp.where(is_b, sc, -jnp.inf), axis=1, keepdims=True)
            e = jnp.exp(sc - jnp.where(is_a, m_a, m_b))
            e_a = jnp.where(is_a, e, 0.0)
            e_b = jnp.where(is_b, e, 0.0)
            l_a = jnp.sum(e_a, axis=1, keepdims=True)
            l_b = jnp.sum(e_b, axis=1, keepdims=True)
            return (e_a + e_b) / jnp.where(is_a, l_a, l_b)

        q, k, v, p, o = {}, {}, {}, {}, {}
        acc = None
        for op, j in order:
            if op == "q":
                q[j] = project(wq_p, j, early_q)
            elif op == "k":
                k[j] = project(wk_p, j, early_k if j < B_EARLY_K else None)
            elif op == "v":
                v[j] = project(wv_p, j)
            elif op == "s":
                p[j] = probabilities(q[j], k[j])
            elif op == "p":
                o[j] = _dot(p[j], block_diag(v[j]))
            else:
                d = _dot(o[j], _unpack(wo_p[j]))
                acc = d if acc is None else acc + d
        out_v[rows, D:] = acc[M:].astype(BF16)
        out_v[rows, :D] = _dot(oa_v[rows, :], _unpack(woa_p[...])).astype(BF16)
        pltpu.make_async_copy(out_v.at[rows], out_hbm.at[rows], sem_o.at[0]).start()
        return acc[:M]

    def b_loop(i, mem):
        for u in range(B_UNROLL):
            mem = b_segment(i * B_UNROLL + u, mem)
        return mem

    lax.fori_loop(0, n_seg // B_UNROLL, b_loop, mem_v[...].astype(F32))

    pltpu.make_async_copy(out_v, out_hbm, sem_o.at[0]).wait()


@functools.partial(jax.jit, static_argnames=("B_seg_len",))
def pallas_concat_heads__sliding_local_dilated__memory_aug_recurrent_mem_tr__prompt_kernel(
    A_x: jax.Array,
    A_wqkv: jax.Array,
    A_wo: jax.Array,
    B_x: jax.Array,
    B_mem0: jax.Array,
    B_Wq: jax.Array,
    B_Wk: jax.Array,
    B_Wv: jax.Array,
    B_Wo: jax.Array,
    B_seg_len: int,
):
    batch, S, D = A_x.shape
    _, H, Dh = B_Wq.shape
    M = B_mem0.shape[1]
    HD = H * Dh
    NP = H // 2
    PW = 2 * Dh
    NT = D // LANES
    n_early = S // B_seg_len * B_EARLY
    assert batch == 1 and B_x.shape == A_x.shape
    assert D % LANES == 0 and PW % LANES == 0 and NT <= A_WIN
    assert S % (2 * A_ROWS) == 0 and S % (B_UNROLL * B_seg_len) == 0
    assert M % 8 == 0 and B_seg_len % 16 == 0 and 2 * (M + B_seg_len) < LANES
    assert NP % B_PAIRS == 0 and NP > 6 and B_EARLY_K <= B_PAIRS

    def heads_major(w):
        return w.transpose(1, 2, 0).reshape(HD, D)

    qkv_set = pltpu.VMEM((3 * NT, A_HALO + A_ROWS, LANES), F32)
    out = pl.pallas_call(
        functools.partial(_kernel, seg=B_seg_len, head_dim=Dh),
        out_shape=jax.ShapeDtypeStruct((S, 2 * D), BF16),
        in_specs=[pl.BlockSpec(memory_space=pltpu.HBM)] * 9,
        out_specs=pl.BlockSpec(memory_space=pltpu.HBM),
        scratch_shapes=[
            pltpu.VMEM((S, D), BF16),
            pltpu.VMEM((3, D, D), BF16),
            pltpu.VMEM((D, D), BF16),
            pltpu.VMEM((NT, D + PERM_PAD, LANES), F32),
            pltpu.VMEM((3 * D // 2, D), U32),
            pltpu.VMEM((D // 2, D), U32),
            qkv_set,
            qkv_set,
            pltpu.VMEM((A_SLOTS, A_WIN, A_GROUP, LANES), F32),
            pltpu.VMEM((S, D), BF16),
            pltpu.VMEM((S, D), BF16),
            pltpu.VMEM((M, D), BF16),
            pltpu.VMEM((HD, D), BF16),
            pltpu.VMEM((HD, D), BF16),
            pltpu.VMEM((HD, D), BF16),
            pltpu.VMEM((HD, D), BF16),
            pltpu.VMEM((NP, D // 2, PW), U32),
            pltpu.VMEM((NP, D // 2, PW), U32),
            pltpu.VMEM((NP, D // 2, PW), U32),
            pltpu.VMEM((NP, PW // 2, D), U32),
            pltpu.VMEM((n_early // 2, D), U32),
            pltpu.VMEM((NP, n_early, PW), F32),
            pltpu.VMEM((B_EARLY_K, n_early, PW), F32),
            pltpu.VMEM((S, 2 * D), BF16),
            pltpu.SemaphoreType.DMA((6,)),
            pltpu.SemaphoreType.DMA((S // (2 * A_ROWS),)),
            pltpu.SemaphoreType.DMA((NP // B_PAIRS,)),
            pltpu.SemaphoreType.DMA((1,)),
        ],
        compiler_params=pltpu.CompilerParams(vmem_limit_bytes=120 * 1024 * 1024),
    )(
        A_x.reshape(S, D), A_wqkv, A_wo, B_x.reshape(S, D), B_mem0.reshape(M, D),
        heads_major(B_Wq), heads_major(B_Wk), heads_major(B_Wv), B_Wo.reshape(HD, D),
    )
    return out.reshape(1, S, 2 * D)
```
